```python
import jax
import jax.numpy as jnp

def _softmax(x, axis=-1):
    return jax.nn.softmax(x, axis=axis)

def _gelu(x):
    return jax.nn.gelu(x, approximate=True)

def _silu(x):
    return jax.nn.silu(x)

def _sigmoid(x):
    return jax.nn.sigmoid(x)

def _layernorm(x, axis=-1, eps=1e-05):
    m = jnp.mean(x, axis=axis, keepdims=True)
    v = jnp.var(x, axis=axis, keepdims=True)
    return (x - m) / jnp.sqrt(v + eps)

def _scatter_add(tgt, idx, src, axis=0):
    return tgt.at[idx].add(src)

def _segment_sum(src, seg, n):
    return jax.ops.segment_sum(src, seg, n)

class _Rng:

    def __init__(self, key):
        self._k = key

    def _next(self):
        self._k, sub = jax.random.split(self._k)
        return sub

    def normal(self, shape):
        return jax.random.normal(self._next(), shape, dtype=jnp.bfloat16)

    def randint(self, lo, hi, shape):
        return jax.random.randint(self._next(), shape, lo, hi, dtype=jnp.int32)

    def uniform(self, shape, lo=0.0, hi=1.0):
        return jax.random.uniform(self._next(), shape, jnp.bfloat16, lo, hi)

    def permutation(self, n):
        return jax.random.permutation(self._next(), n)
kernel_name = 'concat_heads__memory_aug_recurrent_mem_tr__spectral_gfnet__prompt'

def setup_inputs():
    _rng = _Rng(jax.random.key(int.from_bytes(__import__("os").urandom(4), "little")))
    _w = lambda a: (lambda t: t.astype(jnp.bfloat16) if jnp.issubdtype(t.dtype, jnp.floating) else t)(jnp.asarray(a))

    def _A_setup():
        B, S, Dm = (1, 2048, 1024)
        H, Dh = (32, 128)
        M, seg = (8, 32)
        seg = min(seg, S)
        S = S // seg * seg
        return {'x': _w((lambda *s: _rng.normal(s) * 0.05)(B, S, Dm)), 'mem0': _w((lambda *s: _rng.normal(s) * 0.05)(B, M, Dm)), 'Wq': _w((lambda *s: _rng.normal(s) * 0.05)(Dm, H, Dh) * Dm ** (-0.5)), 'Wk': _w((lambda *s: _rng.normal(s) * 0.05)(Dm, H, Dh) * Dm ** (-0.5)), 'Wv': _w((lambda *s: _rng.normal(s) * 0.05)(Dm, H, Dh) * Dm ** (-0.5)), 'Wo': _w((lambda *s: _rng.normal(s) * 0.05)(H, Dh, Dm) * (H * Dh) ** (-0.5)), 'seg_len': seg}
    _A_in = _A_setup()

    def _B_setup():
        B, S, D = (1, 2048, 1024)
        Df = D // 2 + 1
        return {'x': _w((lambda *s: _rng.normal(s) * 0.05)(B, S, D)), 'w_r': _w((lambda *s: _rng.normal(s) * 0.05)(S, Df) * 0.02), 'w_i': _w((lambda *s: _rng.normal(s) * 0.05)(S, Df) * 0.02)}
    _B_in = _B_setup()
    return {'A_x': _A_in['x'], 'A_mem0': _A_in['mem0'], 'A_Wq': _A_in['Wq'], 'A_Wk': _A_in['Wk'], 'A_Wv': _A_in['Wv'], 'A_Wo': _A_in['Wo'], 'A_seg_len': _A_in['seg_len'], 'B_x': _B_in['x'], 'B_w_r': _B_in['w_r'], 'B_w_i': _B_in['w_i']}

def reference(A_x, A_mem0, A_Wq, A_Wk, A_Wv, A_Wo, A_seg_len, B_x, B_w_r, B_w_i):

    def _A_ref(x, mem0, Wq, Wk, Wv, Wo, seg_len):
        B, S, Dm = x.shape
        H, Dh = (Wq.shape[1], Wq.shape[2])
        M = mem0.shape[1]
        scale = Dh ** (-0.5)
        n_seg = S // seg_len
        L = M + seg_len
        idx = jnp.arange(L)
        mask = (idx[:, None] < M) | (idx[:, None] >= idx[None, :])
        mem = mem0
        outs = []
        for s in range(n_seg):
            xs = x[:, s * seg_len:(s + 1) * seg_len, :].copy()
            h = jnp.concatenate([mem, xs], axis=1)
            q = jnp.einsum('btd,dhe->bhte', h, Wq)
            k = jnp.einsum('btd,dhe->bhte', h, Wk)
            v = jnp.einsum('btd,dhe->bhte', h, Wv)
            scores = jnp.einsum('bhqe,bhke->bhqk', q, k) * scale
            scores = jnp.where(mask[None, None], scores, -1000000000.0)
            p = _softmax(scores, axis=-1)
            o = jnp.einsum('bhqk,bhke->bhqe', p, v)
            o = jnp.einsum('bhte,hed->btd', o, Wo)
            mem = o[:, :M, :].copy()
            outs.append(o[:, M:, :])
        return jnp.concatenate(outs, axis=1)

    def _B_ref(x, w_r, w_i):
        B, S, D = x.shape
        X = (lambda x, axes=(-2, -1): jnp.fft.rfft2(x.astype(jnp.float32), axes=axes))(x, axes=(-2, -1))
        W = w_r + 1j * w_i
        X = X * W
        y = (lambda x, s, axes=(-2, -1): jnp.fft.irfft2(x, s=s, axes=axes).astype(jnp.bfloat16))(X, (S, D), axes=(-2, -1))
        return y
    a = _A_ref(A_x, A_mem0, A_Wq, A_Wk, A_Wv, A_Wo, A_seg_len)
    b = _B_ref(B_x, B_w_r, B_w_i)
    return jnp.concatenate([a, b], axis=-1)
```

```python
import functools

import jax
import jax.numpy as jnp
import numpy as np
import jax.experimental.pallas as pl
import jax.experimental.pallas.tpu as pltpu

_F32 = jnp.float32
_BF16 = jnp.bfloat16
_U32 = jnp.uint32

_R = 16
_SQ = float(np.sqrt(0.5))


def _dft_constants(S, D):
    half = D // 2
    d = np.arange(D, dtype=np.int64)
    k = np.arange(half, dtype=np.int64)
    ang = 2.0 * np.pi * ((d[:, None] * k[None, :]) % D) / D
    sign = np.where(d % 2 == 0, 1.0, -1.0)
    nyq = np.zeros((D, 128))
    nyq[:, 0] = sign
    fd = np.concatenate([np.cos(ang), -np.sin(ang), nyq], axis=1)
    c = np.full((half, 1), 2.0)
    c[0, 0] = 1.0
    norm = 1.0 / (S * D)
    fdi = np.concatenate([c * np.cos(ang).T, -c * np.sin(ang).T, nyq.T], axis=0) * norm
    n2 = np.arange(S // _R, dtype=np.int64)
    g = np.zeros((_R, 2 * (S // _R), 2 * (S // _R)))
    for k1 in range(_R):
        freq = k1 + _R * n2
        a = 2.0 * np.pi * ((freq[:, None] * n2[None, :]) % S) / S
        fr, fi = np.cos(a), -np.sin(a)
        g[k1] = np.block([[fr, -fi], [fi, fr]])
    gt = np.ascontiguousarray(g.transpose(0, 2, 1))
    cast = lambda a: np.asarray(a, np.float32).astype(_BF16)
    return cast(fd), cast(fdi), cast(g), cast(gt)


def _cmul_const(z, j, n, sgn):
    re, im = z
    j %= n
    if j == 0:
        return re, im
    if 2 * j == n:
        return -re, -im
    if 4 * j == n:
        return (-im, re) if sgn > 0 else (im, -re)
    if 4 * j == 3 * n:
        return (im, -re) if sgn > 0 else (-im, re)
    c = float(np.cos(2 * np.pi * j / n))
    s = float(sgn * np.sin(2 * np.pi * j / n))
    if 8 * j % n == 0:
        a = re + im if c * s < 0 else re - im
        b = im - re if c * s < 0 else im + re
        return a * c, b * c
    return re * c - im * s, re * s + im * c


def _fft(zs, sgn):
    n = len(zs)
    if n == 1:
        return zs
    ev = _fft(zs[0::2], sgn)
    od = _fft(zs[1::2], sgn)
    out = [None] * n
    for j in range(n // 2):
        if 4 * j == n:
            (er, ei), (orr, oi) = ev[j], od[j]
            if sgn > 0:
                out[j], out[j + n // 2] = (er - oi, ei + orr), (er + oi, ei - orr)
            else:
                out[j], out[j + n // 2] = (er + oi, ei - orr), (er - oi, ei + orr)
            continue
        tr, ti = _cmul_const(od[j], j, n, sgn)
        out[j] = (ev[j][0] + tr, ev[j][1] + ti)
        out[j + n // 2] = (ev[j][0] - tr, ev[j][1] - ti)
    return out


def _kernel(ax_hbm, mem0_ref, wq_hbm, wk_hbm, wv_hbm, wo_hbm, bx_hbm, wr_hbm, wi_hbm,
            fd_hbm, fdi_hbm, g_hbm, gt_hbm, out_hbm,
            ax, stage, wqkv, wo, hbuf, obuf, acc, aout,
            bx, wr, wi, fd, fdi, g, gt, z, bout,
            sem_in, sem_w, sem_ao, sem_bo, *, S, D, H, M, seg):
    half = D // 2
    LW = half + 128
    N2 = S // _R
    L = M + seg
    npair = H // 2
    w_hbms = (wq_hbm, wk_hbm, wv_hbm)

    in_copies = [
        pltpu.make_async_copy(bx_hbm, bx, sem_in.at[0]),
        pltpu.make_async_copy(fd_hbm, fd, sem_in.at[1]),
        pltpu.make_async_copy(g_hbm, g, sem_in.at[2]),
        None,
        None,
        pltpu.make_async_copy(gt_hbm, gt, sem_in.at[5]),
        pltpu.make_async_copy(fdi_hbm, fdi, sem_in.at[6]),
        pltpu.make_async_copy(ax_hbm, ax, sem_in.at[7]),
        pltpu.make_async_copy(wo_hbm.bitcast(_U32), wo, sem_in.at[8]),
    ]

    def w_copy(m, j):
        return pltpu.make_async_copy(w_hbms[m].bitcast(_U32).at[:, j, :],
                                     stage.at[m * npair + j], sem_w.at[m * npair + j])

    f_copies = [pltpu.make_async_copy(src.bitcast(_U32).at[:, a, :], dst.at[a], sem_in.at[3])
                for src, dst in ((wr_hbm, wr), (wi_hbm, wi)) for a in range(_R // 2)]
    for c in in_copies[:3] + f_copies + in_copies[5:7]:
        c.start()
    in_copies[0].wait()
    in_copies[1].wait()
    for m in range(3):
        for j in range(npair):
            w_copy(m, j).start()
    in_copies[8].start()
    in_copies[7].start()

    def fwd_d(n1, _):
        r0 = pl.multiple_of(n1 * N2, N2)
        y = jnp.dot(bx[pl.ds(r0, N2), :], fd[...], preferred_element_type=_F32)
        z[n1, 0:N2, 0:half] = y[:, 0:half]
        z[n1, N2:2 * N2, 0:half] = y[:, half:D]
        z[n1, 0:N2, half:LW] = y[:, D:D + 128]
        z[n1, N2:2 * N2, half:LW] = jnp.zeros((N2, 128), _F32)
        return 0
    jax.lax.fori_loop(0, _R, fwd_d, 0)

    def radix(sgn):
        def body(i, _):
            r0 = pl.multiple_of(i * 8, 8)
            for t in range(LW // 128):
                ls = slice(t * 128, (t + 1) * 128)
                zs = [(z[n, pl.ds(r0, 8), ls], z[n, pl.ds(N2 + r0, 8), ls]) for n in range(_R)]
                ys = _fft(zs, sgn)
                for n in range(_R):
                    z[n, pl.ds(r0, 8), ls] = ys[n][0]
                    z[n, pl.ds(N2 + r0, 8), ls] = ys[n][1]
            return 0
        jax.lax.fori_loop(0, N2 // 8, body, 0)

    radix(-1)
    for c in [in_copies[2], in_copies[5]] + f_copies:
        c.wait()

    lane = jax.lax.broadcasted_iota(jnp.int32, (N2, 128), 1)

    def unpack_w(ref, a):
        u = ref[a, :, 0:half]
        un = jnp.broadcast_to(ref[a, :, half:half + 1], (N2, 128))
        un = jnp.where(lane == 0, un, jnp.uint32(0))
        u = jnp.concatenate([u, un], axis=1)
        return (pltpu.bitcast(u << 16, _F32), pltpu.bitcast(u & jnp.uint32(0xFFFF0000), _F32))

    def mid(a, _):
        wrs = unpack_w(wr, a)
        wis = unpack_w(wi, a)
        for b in range(2):
            k1 = 2 * a + b
            x = jnp.dot(g[k1], z[k1], preferred_element_type=_F32)
            xr, xi = x[0:N2], x[N2:2 * N2]
            y = jnp.concatenate([xr * wrs[b] - xi * wis[b], xr * wis[b] + xi * wrs[b]], axis=0)
            z[k1] = jnp.dot(gt[k1], y, preferred_element_type=_F32)
        return 0
    jax.lax.fori_loop(0, _R // 2, mid, 0)

    radix(+1)
    in_copies[6].wait()

    def bo_copy(n1):
        r0 = pl.multiple_of(n1 * N2, N2)
        return pltpu.make_async_copy(bout.at[pl.ds(r0, N2), :],
                                     out_hbm.at[pl.ds(r0, N2), D:2 * D], sem_bo)

    def inv_d(n1, _):
        r0 = pl.multiple_of(n1 * N2, N2)
        lhs = jnp.concatenate([z[n1, 0:N2, 0:half], z[n1, N2:2 * N2, 0:half],
                               z[n1, 0:N2, half:LW]], axis=1)
        y = jnp.dot(lhs, fdi[...], preferred_element_type=_F32)
        bout[pl.ds(r0, N2), :] = y.astype(_BF16)
        bo_copy(n1).start()
        return 0
    jax.lax.fori_loop(0, _R, inv_d, 0)

    for m in range(3):
        def relayout(j, _, m=m):
            w_copy(m, j).wait()
            u = stage[m * npair + j]
            lo = pltpu.bitcast(u << 16, _F32).astype(_BF16)
            hi = pltpu.bitcast(u & jnp.uint32(0xFFFF0000), _F32).astype(_BF16)
            wqkv[m, 2 * j] = pltpu.bitcast(lo, _U32)
            wqkv[m, 2 * j + 1] = pltpu.bitcast(hi, _U32)
            return 0
        jax.lax.fori_loop(0, npair, relayout, 0)
    in_copies[7].wait()
    in_copies[8].wait()

    hbuf[0:M, :] = mem0_ref[...].astype(_F32)
    hbuf[M:L, :] = ax[0:seg, :].astype(_F32)
    nseg = S // seg
    scale = float(np.asarray(128.0 ** -0.5, np.float32).astype(_BF16).astype(np.float32))
    neg = float(np.asarray(-1e9, np.float32).astype(_BF16).astype(np.float32))

    row = jax.lax.broadcasted_iota(jnp.int32, (2 * L, 128), 0)
    col = jax.lax.broadcasted_iota(jnp.int32, (2 * L, 128), 1)
    rh = (row >= L).astype(jnp.int32)
    ch = (col >= L).astype(jnp.int32) + (col >= 2 * L).astype(jnp.int32)
    tq = row - rh * L
    tk = col - ch * L
    same = rh == ch
    allowed = same & ((tq < M) | (tq >= tk))
    fill = jnp.where(same, jnp.float32(neg), jnp.float32(-np.inf))

    GP = 2
    ngroup = npair // GP

    def qkv_group(gi):
        ws = []
        for p in range(GP):
            for m in range(3):
                for b in range(2):
                    ws.append(wqkv[m, 2 * (gi * GP + p) + b])
        w = pltpu.bitcast(jnp.concatenate(ws, axis=1), _BF16)
        return jnp.dot(hbuf[...], w, preferred_element_type=_F32)

    def attn_group(gi, y):
        zpad = jnp.zeros((128 - 2 * L, 128), _F32)
        for p in range(GP):
            t = [y[:, (6 * p + i) * 128:(6 * p + i + 1) * 128] for i in range(6)]
            q2 = jnp.concatenate([t[0], t[1]], axis=0)
            k2 = jnp.concatenate([t[2], t[3], zpad], axis=0).astype(_BF16)
            v2 = jnp.concatenate([t[4], t[5], zpad], axis=0).astype(_BF16)
            s = jax.lax.dot_general(q2, k2, (((1,), (1,)), ((), ())),
                                    preferred_element_type=_F32)
            s = jnp.where(allowed, s * scale, fill)
            e = jnp.exp(s - jnp.max(s, axis=1, keepdims=True))
            pr = e * pl.reciprocal(jnp.sum(e, axis=1, keepdims=True))
            o = jnp.dot(pr, v2, preferred_element_type=_F32)
            h0 = 2 * (gi * GP + p)
            obuf[:, h0 * 128:(h0 + 1) * 128] = o[0:L]
            obuf[:, (h0 + 1) * 128:(h0 + 2) * 128] = o[L:2 * L]

    def out_group(gi):
        c0, c1 = gi * GP * 256, (gi + 1) * GP * 256
        w = pltpu.bitcast(wo[c0 // 2:c1 // 2, :], _BF16)
        y = jnp.dot(obuf[:, c0:c1], w, preferred_element_type=_F32)
        if gi == 0:
            acc[...] = y
        else:
            acc[...] += y

    def step(s, _):
        for gi in range(ngroup):
            y = qkv_group(gi)
            if gi >= 1:
                out_group(gi - 1)
            attn_group(gi, y)
        nxt = pl.multiple_of(jnp.minimum(s + 1, nseg - 1) * seg, seg)
        hbuf[M:L, :] = ax[pl.ds(nxt, seg), :].astype(_F32)
        out_group(ngroup - 1)
        hbuf[0:M, :] = acc[0:M, :]
        r0 = pl.multiple_of(s * seg, seg)
        aout[pl.ds(r0, seg), :] = acc[M:L, :].astype(_BF16)
        pltpu.make_async_copy(aout.at[pl.ds(r0, seg), :], out_hbm.at[pl.ds(r0, seg), 0:D],
                              sem_ao).start()
        return 0
    jax.lax.fori_loop(0, nseg, step, 0)

    pltpu.make_async_copy(aout, out_hbm.at[:, 0:D], sem_ao).wait()
    pltpu.make_async_copy(bout, out_hbm.at[:, D:2 * D], sem_bo).wait()


@functools.partial(jax.jit, static_argnames=("A_seg_len",))
def pallas_concat_heads__memory_aug_recurrent_mem_tr__spectral_gfnet__prompt_kernel(
    A_x, A_mem0, A_Wq, A_Wk, A_Wv, A_Wo, A_seg_len, B_x, B_w_r, B_w_i,
):
    _, S, D = A_x.shape
    H, Dh = A_Wq.shape[1], A_Wq.shape[2]
    M = A_mem0.shape[1]
    seg = int(A_seg_len)
    assert (S, D, H, Dh, M, seg) == (2048, 1024, 32, 128, 8, 32) and B_x.shape == (1, S, D)
    L = M + seg
    half = D // 2
    N2 = S // _R
    fd, fdi, g, gt = _dft_constants(S, D)

    hbm = pl.BlockSpec(memory_space=pl.ANY)
    vm = pltpu.VMEM
    out = pl.pallas_call(
        functools.partial(_kernel, S=S, D=D, H=H, M=M, seg=seg),
        out_shape=jax.ShapeDtypeStruct((S, 2 * D), _BF16),
        in_specs=[hbm, pl.BlockSpec(memory_space=pltpu.VMEM)] + [hbm] * 11,
        out_specs=hbm,
        scratch_shapes=[
            vm((S, D), _BF16),
            vm((3 * H // 2, D, Dh), _U32),
            vm((3, H, D // 2, Dh), _U32),
            vm((H * Dh // 2, D), _U32),
            vm((L, D), _F32),
            vm((L, H * Dh), _F32),
            vm((L, D), _F32),
            vm((S, D), _BF16),
            vm((S, D), _BF16),
            vm((_R // 2, N2, half + 1), _U32),
            vm((_R // 2, N2, half + 1), _U32),
            vm((D, D + 128), _BF16),
            vm((D + 128, D), _BF16),
            vm((_R, 2 * N2, 2 * N2), _BF16),
            vm((_R, 2 * N2, 2 * N2), _BF16),
            vm((_R, 2 * N2, half + 128), _F32),
            vm((S, D), _BF16),
            pltpu.SemaphoreType.DMA((9,)),
            pltpu.SemaphoreType.DMA((3 * H // 2,)),
            pltpu.SemaphoreType.DMA,
            pltpu.SemaphoreType.DMA,
        ],
        compiler_params=pltpu.CompilerParams(vmem_limit_bytes=120 * 1024 * 1024),
    )(A_x.reshape(S, D), A_mem0.reshape(M, D), A_Wq, A_Wk, A_Wv, A_Wo.reshape(H * Dh, D),
      B_x.reshape(S, D), B_w_r.reshape(N2, _R, half + 1), B_w_i.reshape(N2, _R, half + 1),
      fd, fdi, g, gt)
    return out.reshape(1, S, 2 * D)
```

```python
import functools

import jax
import jax.numpy as jnp
import numpy as np
import jax.experimental.pallas as pl
import jax.experimental.pallas.tpu as pltpu

_F32 = jnp.float32
_BF16 = jnp.bfloat16
_U32 = jnp.uint32

_R = 16
_SQ = float(np.sqrt(0.5))


def _dft_constants(S, D):
    half = D // 2
    d = np.arange(D, dtype=np.int64)
    k = np.arange(half, dtype=np.int64)
    ang = 2.0 * np.pi * ((d[:, None] * k[None, :]) % D) / D
    sign = np.where(d % 2 == 0, 1.0, -1.0)
    nyq = np.zeros((D, 128))
    nyq[:, 0] = sign
    fd = np.concatenate([np.cos(ang), -np.sin(ang), nyq], axis=1)
    c = np.full((half, 1), 2.0)
    c[0, 0] = 1.0
    norm = 1.0 / (S * D)
    fdi = np.concatenate([c * np.cos(ang).T, -c * np.sin(ang).T, nyq.T], axis=0) * norm
    n2 = np.arange(S // _R, dtype=np.int64)
    g = np.zeros((_R, 2 * (S // _R), 2 * (S // _R)))
    for k1 in range(_R):
        freq = k1 + _R * n2
        a = 2.0 * np.pi * ((freq[:, None] * n2[None, :]) % S) / S
        fr, fi = np.cos(a), -np.sin(a)
        g[k1] = np.block([[fr, -fi], [fi, fr]])
    gt = np.ascontiguousarray(g.transpose(0, 2, 1))
    cast = lambda a: np.asarray(a, np.float32).astype(_BF16)
    return cast(fd), cast(fdi), cast(g), cast(gt)


def _cmul_const(z, j, n, sgn):
    re, im = z
    j %= n
    if j == 0:
        return re, im
    if 2 * j == n:
        return -re, -im
    if 4 * j == n:
        return (-im, re) if sgn > 0 else (im, -re)
    if 4 * j == 3 * n:
        return (im, -re) if sgn > 0 else (-im, re)
    c = float(np.cos(2 * np.pi * j / n))
    s = float(sgn * np.sin(2 * np.pi * j / n))
    if 8 * j % n == 0:
        a = re + im if c * s < 0 else re - im
        b = im - re if c * s < 0 else im + re
        return a * c, b * c
    return re * c - im * s, re * s + im * c


def _fft(zs, sgn):
    n = len(zs)
    if n == 1:
        return zs
    ev = _fft(zs[0::2], sgn)
    od = _fft(zs[1::2], sgn)
    out = [None] * n
    for j in range(n // 2):
        if 4 * j == n:
            (er, ei), (orr, oi) = ev[j], od[j]
            if sgn > 0:
                out[j], out[j + n // 2] = (er - oi, ei + orr), (er + oi, ei - orr)
            else:
                out[j], out[j + n // 2] = (er + oi, ei - orr), (er - oi, ei + orr)
            continue
        tr, ti = _cmul_const(od[j], j, n, sgn)
        out[j] = (ev[j][0] + tr, ev[j][1] + ti)
        out[j + n // 2] = (ev[j][0] - tr, ev[j][1] - ti)
    return out


def _kernel(ax_hbm, mem0_ref, wq_hbm, wk_hbm, wv_hbm, wo_hbm, bx_hbm, wr_hbm, wi_hbm,
            fd_hbm, fdi_hbm, g_hbm, gt_hbm, out_hbm,
            ax, stage, wqkv, wo, hbuf, obuf, acc, aout,
            bx, wr, wi, fd, fdi, g, gt, z, bout,
            sem_in, sem_w, sem_ao, sem_bo, *, S, D, H, M, seg):
    half = D // 2
    LW = half + 128
    N2 = S // _R
    L = M + seg
    npair = H // 2
    w_hbms = (wq_hbm, wk_hbm, wv_hbm)

    in_copies = [
        pltpu.make_async_copy(bx_hbm, bx, sem_in.at[0]),
        pltpu.make_async_copy(fd_hbm, fd, sem_in.at[1]),
        pltpu.make_async_copy(g_hbm, g, sem_in.at[2]),
        None,
        None,
        pltpu.make_async_copy(gt_hbm, gt, sem_in.at[5]),
        pltpu.make_async_copy(fdi_hbm, fdi, sem_in.at[6]),
        pltpu.make_async_copy(ax_hbm, ax, sem_in.at[7]),
        pltpu.make_async_copy(wo_hbm.bitcast(_U32), wo, sem_in.at[8]),
    ]

    def w_copy(m, j):
        return pltpu.make_async_copy(w_hbms[m].bitcast(_U32).at[:, j, :],
                                     stage.at[m * npair + j], sem_w.at[m * npair + j])

    f_copies = [pltpu.make_async_copy(src.bitcast(_U32).at[:, a, :], dst.at[a], sem_in.at[3])
                for src, dst in ((wr_hbm, wr), (wi_hbm, wi)) for a in range(_R // 2)]
    for c in in_copies[:3] + f_copies + in_copies[5:7]:
        c.start()
    in_copies[0].wait()
    in_copies[1].wait()
    for m in range(3):
        for j in range(npair):
            w_copy(m, j).start()
    in_copies[8].start()
    in_copies[7].start()

    def fwd_d(n1, _):
        r0 = pl.multiple_of(n1 * N2, N2)
        y = jnp.dot(bx[pl.ds(r0, N2), :], fd[...], preferred_element_type=_F32)
        z[n1, 0:N2, 0:half] = y[:, 0:half]
        z[n1, N2:2 * N2, 0:half] = y[:, half:D]
        z[n1, 0:N2, half:LW] = y[:, D:D + 128]
        z[n1, N2:2 * N2, half:LW] = jnp.zeros((N2, 128), _F32)
        return 0
    jax.lax.fori_loop(0, _R, fwd_d, 0)

    def radix(sgn):
        def body(i, _):
            r0 = pl.multiple_of(i * 8, 8)
            for t in range(LW // 128):
                ls = slice(t * 128, (t + 1) * 128)
                zs = [(z[n, pl.ds(r0, 8), ls], z[n, pl.ds(N2 + r0, 8), ls]) for n in range(_R)]
                ys = _fft(zs, sgn)
                for n in range(_R):
                    z[n, pl.ds(r0, 8), ls] = ys[n][0]
                    z[n, pl.ds(N2 + r0, 8), ls] = ys[n][1]
            return 0
        jax.lax.fori_loop(0, N2 // 8, body, 0)

    radix(-1)
    for c in [in_copies[2], in_copies[5]] + f_copies:
        c.wait()

    lane = jax.lax.broadcasted_iota(jnp.int32, (N2, 128), 1)

    def unpack_w(ref, a):
        u = ref[a, :, 0:half]
        un = jnp.broadcast_to(ref[a, :, half:half + 1], (N2, 128))
        un = jnp.where(lane == 0, un, jnp.uint32(0))
        u = jnp.concatenate([u, un], axis=1)
        return (pltpu.bitcast(u << 16, _F32), pltpu.bitcast(u & jnp.uint32(0xFFFF0000), _F32))

    def mid(a, _):
        wrs = unpack_w(wr, a)
        wis = unpack_w(wi, a)
        for b in range(2):
            k1 = 2 * a + b
            x = jnp.dot(g[k1], z[k1], preferred_element_type=_F32)
            xr, xi = x[0:N2], x[N2:2 * N2]
            y = jnp.concatenate([xr * wrs[b] - xi * wis[b], xr * wis[b] + xi * wrs[b]], axis=0)
            z[k1] = jnp.dot(gt[k1], y, preferred_element_type=_F32)
        return 0
    jax.lax.fori_loop(0, _R // 2, mid, 0)

    radix(+1)
    in_copies[6].wait()

    def bo_copy(n1):
        r0 = pl.multiple_of(n1 * N2, N2)
        return pltpu.make_async_copy(bout.at[pl.ds(r0, N2), :],
                                     out_hbm.at[pl.ds(r0, N2), D:2 * D], sem_bo)

    def inv_d(n1, _):
        r0 = pl.multiple_of(n1 * N2, N2)
        lhs = jnp.concatenate([z[n1, 0:N2, 0:half], z[n1, N2:2 * N2, 0:half],
                               z[n1, 0:N2, half:LW]], axis=1)
        y = jnp.dot(lhs, fdi[...], preferred_element_type=_F32)
        bout[pl.ds(r0, N2), :] = y.astype(_BF16)
        bo_copy(n1).start()
        return 0
    jax.lax.fori_loop(0, _R, inv_d, 0)

    for m in range(3):
        def relayout(j, _, m=m):
            w_copy(m, j).wait()
            u = stage[m * npair + j]
            lo = pltpu.bitcast(u << 16, _F32).astype(_BF16)
            hi = pltpu.bitcast(u & jnp.uint32(0xFFFF0000), _F32).astype(_BF16)
            wqkv[m, 2 * j] = pltpu.bitcast(lo, _U32)
            wqkv[m, 2 * j + 1] = pltpu.bitcast(hi, _U32)
            return 0
        jax.lax.fori_loop(0, npair, relayout, 0)
    in_copies[7].wait()
    in_copies[8].wait()

    hbuf[0:M, :] = mem0_ref[...].astype(_F32)
    hbuf[M:L, :] = ax[0:seg, :].astype(_F32)
    nseg = S // seg
    scale = float(np.asarray(128.0 ** -0.5, np.float32).astype(_BF16).astype(np.float32))
    neg = float(np.asarray(-1e9, np.float32).astype(_BF16).astype(np.float32))

    row = jax.lax.broadcasted_iota(jnp.int32, (L, 128), 0)
    col = jax.lax.broadcasted_iota(jnp.int32, (L, 128), 1)
    allowed = (col < L) & ((row < M) | (row >= col))
    fill = jnp.where(col < L, jnp.float32(neg), jnp.float32(-np.inf))

    G = 4
    ngroup = H // G

    def proj(m, heads):
        w = pltpu.bitcast(jnp.concatenate([wqkv[m, h] for h in heads], axis=1), _BF16)
        y = jnp.dot(hbuf[...], w, preferred_element_type=_F32)
        return [y[:, i * 128:(i + 1) * 128] for i in range(len(heads))]

    def pad_keys(t):
        return jnp.concatenate([t, jnp.zeros((128 - L, 128), _F32)], axis=0).astype(_BF16)

    def probs(q, k):
        s = jax.lax.dot_general(q, pad_keys(k), (((1,), (1,)), ((), ())),
                                preferred_element_type=_F32)
        s = jnp.where(allowed, s * scale, fill)
        e = jnp.exp(s - jnp.max(s, axis=1, keepdims=True))
        den = jnp.sum(e, axis=1, keepdims=True)
        r = pl.reciprocal(den, approx=True)
        return e * (r * (2.0 - den * r))

    def out_part(gi, n0, n1):
        c0, c1 = gi * G * 128, (gi + 1) * G * 128
        w = pltpu.bitcast(wo[c0 // 2:c1 // 2, n0:n1], _BF16)
        y = jnp.dot(obuf[:, c0:c1], w, preferred_element_type=_F32)
        if gi == 0:
            acc[:, n0:n1] = y
        else:
            acc[:, n0:n1] += y

    def group(gi):
        heads = list(range(gi * G, (gi + 1) * G))
        ks = proj(1, heads)
        qs = proj(0, heads)
        vs = proj(2, heads[:2])
        ps = [probs(q, k) for q, k in zip(qs, ks)]
        vs += proj(2, heads[2:])
        if gi >= 1:
            out_part(gi - 1, 0, 640)
        for h, p, v in zip(heads, ps, vs):
            obuf[:, h * 128:(h + 1) * 128] = jnp.dot(p, pad_keys(v), preferred_element_type=_F32)
        if gi >= 1:
            out_part(gi - 1, 640, D)

    def step(s, _):
        for gi in range(ngroup):
            group(gi)
        nxt = pl.multiple_of(jnp.minimum(s + 1, nseg - 1) * seg, seg)
        hbuf[M:L, :] = ax[pl.ds(nxt, seg), :].astype(_F32)
        out_part(ngroup - 1, 0, D)
        hbuf[0:M, :] = acc[0:M, :]
        r0 = pl.multiple_of(s * seg, seg)
        aout[pl.ds(r0, seg), :] = acc[M:L, :].astype(_BF16)
        pltpu.make_async_copy(aout.at[pl.ds(r0, seg), :], out_hbm.at[pl.ds(r0, seg), 0:D],
                              sem_ao).start()
        return 0
    jax.lax.fori_loop(0, nseg, step, 0)

    pltpu.make_async_copy(aout, out_hbm.at[:, 0:D], sem_ao).wait()
    pltpu.make_async_copy(bout, out_hbm.at[:, D:2 * D], sem_bo).wait()


@functools.partial(jax.jit, static_argnames=("A_seg_len",))
def pallas_concat_heads__memory_aug_recurrent_mem_tr__spectral_gfnet__prompt_kernel(
    A_x, A_mem0, A_Wq, A_Wk, A_Wv, A_Wo, A_seg_len, B_x, B_w_r, B_w_i,
):
    _, S, D = A_x.shape
    H, Dh = A_Wq.shape[1], A_Wq.shape[2]
    M = A_mem0.shape[1]
    seg = int(A_seg_len)
    assert (S, D, H, Dh, M, seg) == (2048, 1024, 32, 128, 8, 32) and B_x.shape == (1, S, D)
    L = M + seg
    half = D // 2
    N2 = S // _R
    fd, fdi, g, gt = _dft_constants(S, D)

    hbm = pl.BlockSpec(memory_space=pl.ANY)
    vm = pltpu.VMEM
    out = pl.pallas_call(
        functools.partial(_kernel, S=S, D=D, H=H, M=M, seg=seg),
        out_shape=jax.ShapeDtypeStruct((S, 2 * D), _BF16),
        in_specs=[hbm, pl.BlockSpec(memory_space=pltpu.VMEM)] + [hbm] * 11,
        out_specs=hbm,
        scratch_shapes=[
            vm((S, D), _BF16),
            vm((3 * H // 2, D, Dh), _U32),
            vm((3, H, D // 2, Dh), _U32),
            vm((H * Dh // 2, D), _U32),
            vm((L, D), _F32),
            vm((L, H * Dh), _F32),
            vm((L, D), _F32),
            vm((S, D), _BF16),
            vm((S, D), _BF16),
            vm((_R // 2, N2, half + 1), _U32),
            vm((_R // 2, N2, half + 1), _U32),
            vm((D, D + 128), _BF16),
            vm((D + 128, D), _BF16),
            vm((_R, 2 * N2, 2 * N2), _BF16),
            vm((_R, 2 * N2, 2 * N2), _BF16),
            vm((_R, 2 * N2, half + 128), _F32),
            vm((S, D), _BF16),
            pltpu.SemaphoreType.DMA((9,)),
            pltpu.SemaphoreType.DMA((3 * H // 2,)),
            pltpu.SemaphoreType.DMA,
            pltpu.SemaphoreType.DMA,
        ],
        compiler_params=pltpu.CompilerParams(vmem_limit_bytes=120 * 1024 * 1024),
    )(A_x.reshape(S, D), A_mem0.reshape(M, D), A_Wq, A_Wk, A_Wv, A_Wo.reshape(H * Dh, D),
      B_x.reshape(S, D), B_w_r.reshape(N2, _R, half + 1), B_w_i.reshape(N2, _R, half + 1),
      fd, fdi, g, gt)
    return out.reshape(1, S, 2 * D)
```

```python
import functools

import jax
import jax.numpy as jnp
import numpy as np
import jax.experimental.pallas as pl
import jax.experimental.pallas.tpu as pltpu

_F32 = jnp.float32
_BF16 = jnp.bfloat16
_U32 = jnp.uint32

_R = 16
_SQ = float(np.sqrt(0.5))


def _dft_constants(S, D):
    half, quart = D // 2, D // 4
    d = np.arange(half, dtype=np.int64)
    m = np.arange(quart, dtype=np.int64)
    blocks = []
    for par in range(2):
        ang = 2.0 * np.pi * (((2 * m[:, None] + par) * d[None, :]) % D) / D
        re, im = np.cos(ang), -np.sin(ang)
        if par == 0:
            im[0] = np.where(d % 2 == 0, 1.0, -1.0)
        blocks += [re, im]
    fd = np.concatenate(blocks, axis=0)
    n2 = np.arange(S // _R, dtype=np.int64)
    g = np.zeros((_R, 2 * (S // _R), 2 * (S // _R)))
    for n1 in range(_R):
        a = 2.0 * np.pi * (((n1 + _R * n2)[:, None] * n2[None, :]) % S) / S
        gr, gi = np.cos(a), -np.sin(a)
        g[n1] = np.block([[gr, gi], [-gi, gr]])
    g = g * np.sqrt(2.0 / (S * D))
    cast = lambda a: np.asarray(a, np.float32).astype(_BF16)
    return cast(fd), cast(g)


def _cmul_const(z, j, n, sgn):
    re, im = z
    j %= n
    if j == 0:
        return re, im
    if 2 * j == n:
        return -re, -im
    if 4 * j == n:
        return (-im, re) if sgn > 0 else (im, -re)
    if 4 * j == 3 * n:
        return (im, -re) if sgn > 0 else (-im, re)
    c = float(np.cos(2 * np.pi * j / n))
    s = float(sgn * np.sin(2 * np.pi * j / n))
    if 8 * j % n == 0:
        a = re + im if c * s < 0 else re - im
        b = im - re if c * s < 0 else im + re
        return a * c, b * c
    return re * c - im * s, re * s + im * c


def _fft(zs, sgn):
    n = len(zs)
    if n == 1:
        return zs
    ev = _fft(zs[0::2], sgn)
    od = _fft(zs[1::2], sgn)
    out = [None] * n
    for j in range(n // 2):
        if 4 * j == n:
            (er, ei), (orr, oi) = ev[j], od[j]
            if sgn > 0:
                out[j], out[j + n // 2] = (er - oi, ei + orr), (er + oi, ei - orr)
            else:
                out[j], out[j + n // 2] = (er + oi, ei - orr), (er - oi, ei + orr)
            continue
        tr, ti = _cmul_const(od[j], j, n, sgn)
        out[j] = (ev[j][0] + tr, ev[j][1] + ti)
        out[j + n // 2] = (ev[j][0] - tr, ev[j][1] - ti)
    return out


def _halves(u):
    return (pltpu.bitcast(u << 16, _F32), pltpu.bitcast(u & jnp.uint32(0xFFFF0000), _F32))


def _kernel(ax_hbm, mem0_ref, wq_hbm, wk_hbm, wv_hbm, wo_hbm, bx_hbm, wr_hbm, wi_hbm,
            wrn_ref, win_ref, fd_hbm, g_hbm, out_hbm,
            ax, stage, wqkv, wo, hbuf, obuf, acc, aout,
            bx, wr, wi, fd, g, z,
            sem_in, sem_x, sem_w, sem_ao, sem_bo, *, S, D, H, M, seg):
    half, quart = D // 2, D // 4
    N2 = S // _R
    L = M + seg
    npair = H // 2
    w_hbms = (wq_hbm, wk_hbm, wv_hbm)
    nt = (((1,), (1,)), ((), ()))
    tn = (((0,), (0,)), ((), ()))

    in_copies = [
        pltpu.make_async_copy(fd_hbm, fd, sem_in.at[0]),
        pltpu.make_async_copy(g_hbm, g, sem_in.at[1]),
        pltpu.make_async_copy(wr_hbm.at[0:half].bitcast(_U32), wr, sem_in.at[2]),
        pltpu.make_async_copy(wi_hbm.at[0:half].bitcast(_U32), wi, sem_in.at[3]),
        pltpu.make_async_copy(wo_hbm.bitcast(_U32), wo, sem_in.at[4]),
        pltpu.make_async_copy(ax_hbm, ax, sem_in.at[5]),
    ]

    def x_copy(a):
        return pltpu.make_async_copy(bx_hbm.bitcast(_U32).at[:, a, :], bx.at[a], sem_x.at[a])

    def w_copy(m, j):
        return pltpu.make_async_copy(w_hbms[m].bitcast(_U32).at[:, j, :],
                                     stage.at[m * npair + j], sem_w.at[m * npair + j])

    x_copy(0).start()
    in_copies[0].start()
    for a in range(1, _R // 2):
        x_copy(a).start()
    for c in in_copies[1:4]:
        c.start()
    for j in range(npair):
        for m in range(3):
            w_copy(m, j).start()
    in_copies[4].start()
    in_copies[5].start()

    first = jax.lax.broadcasted_iota(jnp.int32, (8, N2), 0) == 0
    in_copies[0].wait()

    def fwd_d(a, _):
        x_copy(a).wait()
        for b, x in enumerate(_halves(bx[a])):
            n1 = 2 * a + b
            xe, xo = x[:, 0:half] + x[:, half:D], x[:, 0:half] - x[:, half:D]
            ye = jax.lax.dot_general(fd[0:half, :], xe.astype(_BF16), nt,
                                     preferred_element_type=_F32)
            yo = jax.lax.dot_general(fd[half:D, :], xo.astype(_BF16), nt,
                                     preferred_element_type=_F32)
            z[n1, 0:quart, 0:N2] = ye[0:quart]
            z[n1, 0:8, N2:2 * N2] = jnp.where(first, 0.0, ye[quart:quart + 8])
            z[n1, 8:quart, N2:2 * N2] = ye[quart + 8:half]
            z[n1, quart:half, 0:N2] = yo[0:quart]
            z[n1, quart:half, N2:2 * N2] = yo[quart:half]
            z[n1, half:half + 8, 0:N2] = jnp.where(first, ye[quart:quart + 8], 0.0)
            z[n1, half:half + 8, N2:2 * N2] = jnp.zeros((8, N2), _F32)
        return 0
    jax.lax.fori_loop(0, _R // 2, fwd_d, 0)

    in_copies[1].wait()

    def fwd_s(n1, _):
        z[n1] = jnp.dot(z[n1], g[n1], preferred_element_type=_F32)
        return 0
    jax.lax.fori_loop(0, _R, fwd_s, 0)

    in_copies[2].wait()
    in_copies[3].wait()

    def filt(rows, ws):
        xs = _fft([(z[n, rows, 0:N2], z[n, rows, N2:2 * N2]) for n in range(_R)], -1)
        ys = [(xr * fr - xi * fi, xr * fi + xi * fr) for (xr, xi), (fr, fi) in zip(xs, ws)]
        for n, (yr, yi) in enumerate(_fft(ys, +1)):
            z[n, rows, 0:N2] = yr
            z[n, rows, N2:2 * N2] = yi

    def mid(j, _):
        r0 = pl.multiple_of(j * 8, 8)
        dc = jnp.where(first & (j == 0), 0.5, 1.0)
        for par in range(2):
            ws = []
            for l1 in range(_R):
                ls = slice(l1 * N2, (l1 + 1) * N2)
                fr = _halves(wr[pl.ds(r0, 8), ls])[par]
                fi = _halves(wi[pl.ds(r0, 8), ls])[par]
                ws.append((fr * dc, fi * dc) if par == 0 else (fr, fi))
            filt(pl.ds(par * quart + r0, 8), ws)
        return 0
    jax.lax.fori_loop(0, quart // 8, mid, 0)

    def nyq_w(ref, l1):
        return jnp.where(first, ref[0:8, l1 * N2:(l1 + 1) * N2].astype(_F32) * 0.5, 0.0)
    filt(pl.ds(half, 8), [(nyq_w(wrn_ref, l1), nyq_w(win_ref, l1)) for l1 in range(_R)])

    def inv_s(n1, _):
        z[n1] = jax.lax.dot_general(z[n1], g[n1], nt, preferred_element_type=_F32)
        return 0
    jax.lax.fori_loop(0, _R, inv_s, 0)

    def inv_d(a, _):
        ys = []
        for b in range(2):
            n1 = 2 * a + b
            top = jnp.where(first, z[n1, half:half + 8, 0:N2], z[n1, 0:8, N2:2 * N2])
            ue = jnp.concatenate([z[n1, 0:quart, 0:N2], top, z[n1, 8:quart, N2:2 * N2]], axis=0)
            uo = jnp.concatenate([z[n1, quart:half, 0:N2], z[n1, quart:half, N2:2 * N2]], axis=0)
            p = jax.lax.dot_general(ue, fd[0:half, :], tn, preferred_element_type=_F32)
            q = jax.lax.dot_general(uo, fd[half:D, :], tn, preferred_element_type=_F32)
            ys.append(jnp.concatenate([p + q, p - q], axis=1))
        bx[a] = pltpu.bitcast(pltpu.pack_elementwise(ys, packed_dtype=_BF16), _U32)
        pltpu.make_async_copy(bx.at[a], out_hbm.bitcast(_U32).at[:, a, D:2 * D], sem_bo).start()
        return 0
    jax.lax.fori_loop(0, _R // 2, inv_d, 0)

    for m in range(3):
        def relayout(j, _, m=m):
            w_copy(m, j).wait()
            u = stage[m * npair + j]
            lo = pltpu.bitcast(u << 16, _F32).astype(_BF16)
            hi = pltpu.bitcast(u & jnp.uint32(0xFFFF0000), _F32).astype(_BF16)
            wqkv[m, 2 * j] = pltpu.bitcast(lo, _U32)
            wqkv[m, 2 * j + 1] = pltpu.bitcast(hi, _U32)
            return 0
        jax.lax.fori_loop(0, npair, relayout, 0)
    in_copies[4].wait()
    in_copies[5].wait()

    hbuf[0:M, :] = mem0_ref[...].astype(_F32)
    hbuf[M:L, :] = ax[0:seg, :].astype(_F32)
    nseg = S // seg
    scale = float(np.asarray(128.0 ** -0.5, np.float32).astype(_BF16).astype(np.float32))
    neg = float(np.asarray(-1e9, np.float32).astype(_BF16).astype(np.float32))

    row = jax.lax.broadcasted_iota(jnp.int32, (L, 128), 0)
    col = jax.lax.broadcasted_iota(jnp.int32, (L, 128), 1)
    allowed = (col < L) & ((row < M) | (row >= col))
    fill = jnp.where(col < L, jnp.float32(neg), jnp.float32(-np.inf))

    G = 4
    ngroup = H // G

    def proj(m, heads):
        w = pltpu.bitcast(jnp.concatenate([wqkv[m, h] for h in heads], axis=1), _BF16)
        y = jnp.dot(hbuf[...], w, preferred_element_type=_F32)
        return [y[:, i * 128:(i + 1) * 128] for i in range(len(heads))]

    def pad_keys(t):
        return jnp.concatenate([t, jnp.zeros((128 - L, 128), _F32)], axis=0).astype(_BF16)

    def probs(q, k):
        s = jax.lax.dot_general(q, pad_keys(k), (((1,), (1,)), ((), ())),
                                preferred_element_type=_F32)
        s = jnp.where(allowed, s * scale, fill)
        e = jnp.exp(s - jnp.max(s, axis=1, keepdims=True))
        den = jnp.sum(e, axis=1, keepdims=True)
        r = pl.reciprocal(den, approx=True)
        return e * (r * (2.0 - den * r))

    def out_part(gi, n0, n1):
        c0, c1 = gi * G * 128, (gi + 1) * G * 128
        w = pltpu.bitcast(wo[c0 // 2:c1 // 2, n0:n1], _BF16)
        y = jnp.dot(obuf[:, c0:c1], w, preferred_element_type=_F32)
        if gi == 0:
            acc[:, n0:n1] = y
        else:
            acc[:, n0:n1] += y

    def group(gi):
        heads = list(range(gi * G, (gi + 1) * G))
        ks = proj(1, heads)
        qs = proj(0, heads)
        vs = proj(2, heads[:2])
        ps = [probs(q, k) for q, k in zip(qs, ks)]
        vs += proj(2, heads[2:])
        if gi >= 1:
            out_part(gi - 1, 0, 640)
        for h, p, v in zip(heads, ps, vs):
            obuf[:, h * 128:(h + 1) * 128] = jnp.dot(p, pad_keys(v), preferred_element_type=_F32)
        if gi >= 1:
            out_part(gi - 1, 640, D)

    def step(s, _):
        for gi in range(ngroup):
            group(gi)
        nxt = pl.multiple_of(jnp.minimum(s + 1, nseg - 1) * seg, seg)
        hbuf[M:L, :] = ax[pl.ds(nxt, seg), :].astype(_F32)
        out_part(ngroup - 1, 0, D)
        hbuf[0:M, :] = acc[0:M, :]
        nb = seg // _R
        for i in range(nb):
            aout[s * nb + i] = acc[M + i * _R:M + (i + 1) * _R, :].astype(_BF16)
        pltpu.make_async_copy(aout.at[pl.ds(s * nb, nb)], out_hbm.at[pl.ds(s * nb, nb), :, 0:D],
                              sem_ao).start()
        return 0
    jax.lax.fori_loop(0, nseg, step, 0)

    pltpu.make_async_copy(aout, out_hbm.at[:, :, 0:D], sem_ao).wait()
    for a in range(_R // 2):
        pltpu.make_async_copy(bx.at[a], out_hbm.bitcast(_U32).at[:, a, D:2 * D], sem_bo).wait()


@functools.partial(jax.jit, static_argnames=("A_seg_len",))
def pallas_concat_heads__memory_aug_recurrent_mem_tr__spectral_gfnet__prompt_kernel(
    A_x, A_mem0, A_Wq, A_Wk, A_Wv, A_Wo, A_seg_len, B_x, B_w_r, B_w_i,
):
    _, S, D = A_x.shape
    H, Dh = A_Wq.shape[1], A_Wq.shape[2]
    M = A_mem0.shape[1]
    seg = int(A_seg_len)
    assert (S, D, H, Dh, M, seg) == (2048, 1024, 32, 128, 8, 32) and B_x.shape == (1, S, D)
    L = M + seg
    half = D // 2
    N2 = S // _R
    fd, g = _dft_constants(S, D)
    wr_t, wi_t = B_w_r.T, B_w_i.T
    nyq = pl.BlockSpec((16, S), lambda i: (half // 16, 0))

    hbm = pl.BlockSpec(memory_space=pl.ANY)
    vm = pltpu.VMEM
    out = pl.pallas_call(
        functools.partial(_kernel, S=S, D=D, H=H, M=M, seg=seg),
        out_shape=jax.ShapeDtypeStruct((N2, _R, 2 * D), _BF16),
        grid=(1,),
        in_specs=[hbm, pl.BlockSpec(memory_space=pltpu.VMEM)] + [hbm] * 7 + [nyq, nyq, hbm, hbm],
        out_specs=hbm,
        scratch_shapes=[
            vm((S, D), _BF16),
            vm((3 * H // 2, D, Dh), _U32),
            vm((3, H, D // 2, Dh), _U32),
            vm((H * Dh // 2, D), _U32),
            vm((L, D), _F32),
            vm((L, H * Dh), _F32),
            vm((L, D), _F32),
            vm((N2, _R, D), _BF16),
            vm((_R // 2, N2, D), _U32),
            vm((half // 2, S), _U32),
            vm((half // 2, S), _U32),
            vm((D, half), _BF16),
            vm((_R, 2 * N2, 2 * N2), _BF16),
            vm((_R, half + 8, 2 * N2), _F32),
            pltpu.SemaphoreType.DMA((6,)),
            pltpu.SemaphoreType.DMA((_R // 2,)),
            pltpu.SemaphoreType.DMA((3 * H // 2,)),
            pltpu.SemaphoreType.DMA,
            pltpu.SemaphoreType.DMA,
        ],
        compiler_params=pltpu.CompilerParams(vmem_limit_bytes=120 * 1024 * 1024),
    )(A_x.reshape(S, D), A_mem0.reshape(M, D), A_Wq, A_Wk, A_Wv, A_Wo.reshape(H * Dh, D),
      B_x.reshape(N2, _R, D), wr_t, wi_t, wr_t, wi_t, fd, g)
    return out.reshape(1, S, 2 * D)
```

```python
import functools

import jax
import jax.numpy as jnp
import numpy as np
import jax.experimental.pallas as pl
import jax.experimental.pallas.tpu as pltpu

_F32 = jnp.float32
_BF16 = jnp.bfloat16
_U32 = jnp.uint32

_R = 16
_SQ = float(np.sqrt(0.5))


def _dft_constants(S, D):
    half, quart = D // 2, D // 4
    d = np.arange(half, dtype=np.int64)
    m = np.arange(quart, dtype=np.int64)
    blocks = []
    for par in range(2):
        ang = 2.0 * np.pi * (((2 * m[:, None] + par) * d[None, :]) % D) / D
        re, im = np.cos(ang), -np.sin(ang)
        if par == 0:
            im[0] = np.where(d % 2 == 0, 1.0, -1.0)
        blocks += [re, im]
    fd = np.concatenate(blocks, axis=0)
    n2 = np.arange(S // _R, dtype=np.int64)
    g = np.zeros((_R, 2 * (S // _R), 2 * (S // _R)))
    for n1 in range(_R):
        a = 2.0 * np.pi * (((n1 + _R * n2)[:, None] * n2[None, :]) % S) / S
        gr, gi = np.cos(a), -np.sin(a)
        g[n1] = np.block([[gr, gi], [-gi, gr]])
    g = g * np.sqrt(2.0 / (S * D))
    cast = lambda a: np.asarray(a, np.float32).astype(_BF16)
    return cast(fd), cast(g)


def _cmul_const(z, j, n, sgn):
    re, im = z
    j %= n
    if j == 0:
        return re, im
    if 2 * j == n:
        return -re, -im
    if 4 * j == n:
        return (-im, re) if sgn > 0 else (im, -re)
    if 4 * j == 3 * n:
        return (im, -re) if sgn > 0 else (-im, re)
    c = float(np.cos(2 * np.pi * j / n))
    s = float(sgn * np.sin(2 * np.pi * j / n))
    if 8 * j % n == 0:
        a = re + im if c * s < 0 else re - im
        b = im - re if c * s < 0 else im + re
        return a * c, b * c
    return re * c - im * s, re * s + im * c


def _fft(zs, sgn):
    n = len(zs)
    if n == 1:
        return zs
    ev = _fft(zs[0::2], sgn)
    od = _fft(zs[1::2], sgn)
    out = [None] * n
    for j in range(n // 2):
        if 4 * j == n:
            (er, ei), (orr, oi) = ev[j], od[j]
            if sgn > 0:
                out[j], out[j + n // 2] = (er - oi, ei + orr), (er + oi, ei - orr)
            else:
                out[j], out[j + n // 2] = (er + oi, ei - orr), (er - oi, ei + orr)
            continue
        tr, ti = _cmul_const(od[j], j, n, sgn)
        out[j] = (ev[j][0] + tr, ev[j][1] + ti)
        out[j + n // 2] = (ev[j][0] - tr, ev[j][1] - ti)
    return out


def _halves(u):
    return (pltpu.bitcast(u << 16, _F32), pltpu.bitcast(u & jnp.uint32(0xFFFF0000), _F32))


def _kernel(ax_hbm, mem0_ref, wq_hbm, wk_hbm, wv_hbm, wo_hbm, bx_hbm, wr_hbm, wi_hbm,
            wrn_ref, win_ref, fd_hbm, g_hbm, out_hbm,
            ax, stage, wqkv, wo, hbuf, obuf, acc, aout,
            bx, wr, wi, fd, g, z,
            sem_in, sem_x, sem_w, sem_wo, sem_ao, sem_bo, *, S, D, H, M, seg):
    half, quart = D // 2, D // 4
    N2 = S // _R
    L = M + seg
    npair = H // 2
    w_hbms = (wq_hbm, wk_hbm, wv_hbm)
    nt = (((1,), (1,)), ((), ()))
    tn = (((0,), (0,)), ((), ()))

    in_copies = [
        pltpu.make_async_copy(fd_hbm, fd, sem_in.at[0]),
        pltpu.make_async_copy(g_hbm, g, sem_in.at[1]),
        pltpu.make_async_copy(wr_hbm.at[0:half].bitcast(_U32), wr, sem_in.at[2]),
        pltpu.make_async_copy(wi_hbm.at[0:half].bitcast(_U32), wi, sem_in.at[3]),
        pltpu.make_async_copy(ax_hbm.at[0:4 * seg], ax.at[0:4 * seg], sem_in.at[4]),
        pltpu.make_async_copy(ax_hbm.at[4 * seg:S], ax.at[4 * seg:S], sem_in.at[5]),
    ]
    G = 4
    ngroup = H // G

    def wo_copy(gi):
        rows = pl.ds(pl.multiple_of(gi * G * 64, G * 64), G * 64)
        return pltpu.make_async_copy(wo_hbm.bitcast(_U32).at[rows], wo.at[rows], sem_wo.at[gi])

    def bo_copy(a):
        return pltpu.make_async_copy(bx.at[a], out_hbm.bitcast(_U32).at[:, a, D:2 * D], sem_bo)

    def x_copy(a):
        return pltpu.make_async_copy(bx_hbm.bitcast(_U32).at[:, a, :], bx.at[a], sem_x.at[a])

    def w_copy(m, j):
        return pltpu.make_async_copy(w_hbms[m].bitcast(_U32).at[:, j, :],
                                     stage.at[m * npair + j], sem_w.at[m * npair + j])

    x_copy(0).start()
    in_copies[0].start()
    for a in range(1, _R // 2):
        x_copy(a).start()
    for c in in_copies[1:4]:
        c.start()
    in_copies[4].start()
    for gi in range(ngroup):
        for j in range(gi * G // 2, (gi + 1) * G // 2):
            for m in range(3):
                w_copy(m, j).start()
        wo_copy(gi).start()

    first = jax.lax.broadcasted_iota(jnp.int32, (8, N2), 0) == 0
    in_copies[0].wait()

    def fwd_d(a, _):
        x_copy(a).wait()
        for b, x in enumerate(_halves(bx[a])):
            n1 = 2 * a + b
            xe, xo = x[:, 0:half] + x[:, half:D], x[:, 0:half] - x[:, half:D]
            ye = jax.lax.dot_general(fd[0:half, :], xe.astype(_BF16), nt,
                                     preferred_element_type=_F32)
            yo = jax.lax.dot_general(fd[half:D, :], xo.astype(_BF16), nt,
                                     preferred_element_type=_F32)
            z[n1, 0:quart, 0:N2] = ye[0:quart]
            z[n1, 0:8, N2:2 * N2] = jnp.where(first, 0.0, ye[quart:quart + 8])
            z[n1, 8:quart, N2:2 * N2] = ye[quart + 8:half]
            z[n1, quart:half, 0:N2] = yo[0:quart]
            z[n1, quart:half, N2:2 * N2] = yo[quart:half]
            z[n1, half:half + 8, 0:N2] = jnp.where(first, ye[quart:quart + 8], 0.0)
            z[n1, half:half + 8, N2:2 * N2] = jnp.zeros((8, N2), _F32)
        return 0
    jax.lax.fori_loop(0, _R // 2, fwd_d, 0)

    in_copies[1].wait()

    def fwd_s(n1, _):
        z[n1] = jnp.dot(z[n1], g[n1], preferred_element_type=_F32)
        return 0
    jax.lax.fori_loop(0, _R, fwd_s, 0)

    in_copies[2].wait()
    in_copies[3].wait()

    def filt(rows, ws):
        xs = _fft([(z[n, rows, 0:N2], z[n, rows, N2:2 * N2]) for n in range(_R)], -1)
        ys = [(xr * fr - xi * fi, xr * fi + xi * fr) for (xr, xi), (fr, fi) in zip(xs, ws)]
        for n, (yr, yi) in enumerate(_fft(ys, +1)):
            z[n, rows, 0:N2] = yr
            z[n, rows, N2:2 * N2] = yi

    def mid(j, _):
        r0 = pl.multiple_of(j * 8, 8)
        dc = jnp.where(first & (j == 0), 0.5, 1.0)
        for par in range(2):
            ws = []
            for l1 in range(_R):
                ls = slice(l1 * N2, (l1 + 1) * N2)
                fr = _halves(wr[pl.ds(r0, 8), ls])[par]
                fi = _halves(wi[pl.ds(r0, 8), ls])[par]
                ws.append((fr * dc, fi * dc) if par == 0 else (fr, fi))
            filt(pl.ds(par * quart + r0, 8), ws)
        return 0
    jax.lax.fori_loop(0, quart // 8, mid, 0)

    def nyq_w(ref, l1):
        return jnp.where(first, ref[0:8, l1 * N2:(l1 + 1) * N2].astype(_F32) * 0.5, 0.0)
    filt(pl.ds(half, 8), [(nyq_w(wrn_ref, l1), nyq_w(win_ref, l1)) for l1 in range(_R)])

    def inv_s(n1, _):
        z[n1] = jax.lax.dot_general(z[n1], g[n1], nt, preferred_element_type=_F32)
        return 0
    jax.lax.fori_loop(0, _R, inv_s, 0)

    def inv_d(a, _):
        ys = []
        for b in range(2):
            n1 = 2 * a + b
            top = jnp.where(first, z[n1, half:half + 8, 0:N2], z[n1, 0:8, N2:2 * N2])
            ue = jnp.concatenate([z[n1, 0:quart, 0:N2], top, z[n1, 8:quart, N2:2 * N2]], axis=0)
            uo = jnp.concatenate([z[n1, quart:half, 0:N2], z[n1, quart:half, N2:2 * N2]], axis=0)
            p = jax.lax.dot_general(ue, fd[0:half, :], tn, preferred_element_type=_F32)
            q = jax.lax.dot_general(uo, fd[half:D, :], tn, preferred_element_type=_F32)
            ys.append(jnp.concatenate([p + q, p - q], axis=1))
        bx[a] = pltpu.bitcast(pltpu.pack_elementwise(ys, packed_dtype=_BF16), _U32)
        return 0
    jax.lax.fori_loop(0, _R // 2, inv_d, 0)

    in_copies[4].wait()
    hbuf[0:M, :] = mem0_ref[...].astype(_F32)
    hbuf[M:L, :] = ax[0:seg, :].astype(_F32)
    nseg = S // seg
    scale = float(np.asarray(128.0 ** -0.5, np.float32).astype(_BF16).astype(np.float32))
    neg = float(np.asarray(-1e9, np.float32).astype(_BF16).astype(np.float32))

    row = jax.lax.broadcasted_iota(jnp.int32, (L, 128), 0)
    col = jax.lax.broadcasted_iota(jnp.int32, (L, 128), 1)
    allowed = (col < L) & ((row < M) | (row >= col))
    fill = jnp.where(col < L, jnp.float32(neg), jnp.float32(-np.inf))

    def proj(m, heads):
        w = pltpu.bitcast(jnp.concatenate([wqkv[m, h] for h in heads], axis=1), _BF16)
        y = jnp.dot(hbuf[...], w, preferred_element_type=_F32)
        return [y[:, i * 128:(i + 1) * 128] for i in range(len(heads))]

    def pad_keys(t):
        return jnp.concatenate([t, jnp.zeros((128 - L, 128), _F32)], axis=0).astype(_BF16)

    def probs(q, k):
        s = jax.lax.dot_general(q, pad_keys(k), (((1,), (1,)), ((), ())),
                                preferred_element_type=_F32)
        s = jnp.where(allowed, s * scale, fill)
        e = jnp.exp(s - jnp.max(s, axis=1, keepdims=True))
        den = jnp.sum(e, axis=1, keepdims=True)
        r = pl.reciprocal(den, approx=True)
        return e * (r * (2.0 - den * r))

    def out_part(gi, n0, n1):
        c0, c1 = gi * G * 128, (gi + 1) * G * 128
        w = pltpu.bitcast(wo[c0 // 2:c1 // 2, n0:n1], _BF16)
        y = jnp.dot(obuf[:, c0:c1], w, preferred_element_type=_F32)
        if gi == 0:
            acc[:, n0:n1] = y
        else:
            acc[:, n0:n1] += y

    def values(heads, ps, vs):
        for h, p, v in zip(heads, ps, vs):
            obuf[:, h * 128:(h + 1) * 128] = jnp.dot(p, pad_keys(v), preferred_element_type=_F32)

    def group(gi, late):
        heads = list(range(gi * G, (gi + 1) * G))
        ks = proj(1, heads)
        if late is not None:
            values(*late)
        qs = proj(0, heads)
        vs = proj(2, heads[:2])
        ps = [probs(q, k) for q, k in zip(qs, ks)]
        vs += proj(2, heads[2:])
        if gi == 0:
            return heads, ps, vs
        out_part(gi - 1, 0, 768)
        values(heads, ps, vs)
        out_part(gi - 1, 768, D)

    def finish(s):
        hbuf[0:M, :] = acc[0:M, :]
        nb = seg // _R
        for i in range(nb):
            aout[s * nb + i] = acc[M + i * _R:M + (i + 1) * _R, :].astype(_BF16)
        pltpu.make_async_copy(aout.at[pl.ds(s * nb, nb)], out_hbm.at[pl.ds(s * nb, nb), :, 0:D],
                              sem_ao).start()

    acc[...] = jnp.zeros((L, D), _F32)

    def first_group(gi, _):
        for jj in range(G // 2):
            j = gi * (G // 2) + jj
            for m in range(3):
                w_copy(m, j).wait()
                for b, w in enumerate(_halves(stage[m * npair + j])):
                    wqkv[m, 2 * j + b] = pltpu.bitcast(w.astype(_BF16), _U32)
        heads = [gi * G + i for i in range(G)]
        ks, qs, vs = proj(1, heads), proj(0, heads), proj(2, heads)
        o = jnp.concatenate([jnp.dot(probs(q, k), pad_keys(v), preferred_element_type=_F32)
                             for q, k, v in zip(qs, ks, vs)], axis=1)
        wo_copy(gi).wait()
        rows = pl.ds(pl.multiple_of(gi * G * 64, G * 64), G * 64)
        acc[...] += jnp.dot(o, pltpu.bitcast(wo[rows, :], _BF16), preferred_element_type=_F32)
        return 0
    jax.lax.fori_loop(0, ngroup, first_group, 0)
    in_copies[5].start()
    hbuf[M:L, :] = ax[seg:2 * seg, :].astype(_F32)
    finish(0)

    def step(s, _):
        @pl.when(s == 3)
        def _():
            in_copies[5].wait()
            for a in range(_R // 2):
                bo_copy(a).start()
        late = None
        for gi in range(ngroup):
            late = group(gi, late)
        nxt = pl.multiple_of(jnp.minimum(s + 1, nseg - 1) * seg, seg)
        hbuf[M:L, :] = ax[pl.ds(nxt, seg), :].astype(_F32)
        out_part(ngroup - 1, 0, D)
        finish(s)
        return 0
    jax.lax.fori_loop(1, nseg, step, 0)

    pltpu.make_async_copy(aout, out_hbm.at[:, :, 0:D], sem_ao).wait()
    for a in range(_R // 2):
        bo_copy(a).wait()


@functools.partial(jax.jit, static_argnames=("A_seg_len",))
def pallas_concat_heads__memory_aug_recurrent_mem_tr__spectral_gfnet__prompt_kernel(
    A_x, A_mem0, A_Wq, A_Wk, A_Wv, A_Wo, A_seg_len, B_x, B_w_r, B_w_i,
):
    _, S, D = A_x.shape
    H, Dh = A_Wq.shape[1], A_Wq.shape[2]
    M = A_mem0.shape[1]
    seg = int(A_seg_len)
    assert (S, D, H, Dh, M, seg) == (2048, 1024, 32, 128, 8, 32) and B_x.shape == (1, S, D)
    L = M + seg
    half = D // 2
    N2 = S // _R
    fd, g = _dft_constants(S, D)
    wr_t, wi_t = B_w_r.T, B_w_i.T
    nyq = pl.BlockSpec((16, S), lambda i: (half // 16, 0))

    hbm = pl.BlockSpec(memory_space=pl.ANY)
    vm = pltpu.VMEM
    out = pl.pallas_call(
        functools.partial(_kernel, S=S, D=D, H=H, M=M, seg=seg),
        out_shape=jax.ShapeDtypeStruct((N2, _R, 2 * D), _BF16),
        grid=(1,),
        in_specs=[hbm, pl.BlockSpec(memory_space=pltpu.VMEM)] + [hbm] * 7 + [nyq, nyq, hbm, hbm],
        out_specs=hbm,
        scratch_shapes=[
            vm((S, D), _BF16),
            vm((3 * H // 2, D, Dh), _U32),
            vm((3, H, D // 2, Dh), _U32),
            vm((H * Dh // 2, D), _U32),
            vm((L, D), _F32),
            vm((L, H * Dh), _F32),
            vm((L, D), _F32),
            vm((N2, _R, D), _BF16),
            vm((_R // 2, N2, D), _U32),
            vm((half // 2, S), _U32),
            vm((half // 2, S), _U32),
            vm((D, half), _BF16),
            vm((_R, 2 * N2, 2 * N2), _BF16),
            vm((_R, half + 8, 2 * N2), _F32),
            pltpu.SemaphoreType.DMA((6,)),
            pltpu.SemaphoreType.DMA((_R // 2,)),
            pltpu.SemaphoreType.DMA((3 * H // 2,)),
            pltpu.SemaphoreType.DMA((H // 4,)),
            pltpu.SemaphoreType.DMA,
            pltpu.SemaphoreType.DMA,
        ],
        compiler_params=pltpu.CompilerParams(vmem_limit_bytes=120 * 1024 * 1024),
    )(A_x.reshape(S, D), A_mem0.reshape(M, D), A_Wq, A_Wk, A_Wv, A_Wo.reshape(H * Dh, D),
      B_x.reshape(N2, _R, D), wr_t, wi_t, wr_t, wi_t, fd, g)
    return out.reshape(1, S, 2 * D)
```

```python
import functools

import jax
import jax.numpy as jnp
import numpy as np
import jax.experimental.pallas as pl
import jax.experimental.pallas.tpu as pltpu

_F32 = jnp.float32
_BF16 = jnp.bfloat16
_U32 = jnp.uint32

_R = 16
_NPRE = 1
_SQ = float(np.sqrt(0.5))


def _dft_constants(S, D):
    half, quart = D // 2, D // 4
    d = np.arange(half, dtype=np.int64)
    m = np.arange(quart, dtype=np.int64)
    blocks = []
    for par in range(2):
        ang = 2.0 * np.pi * (((2 * m[:, None] + par) * d[None, :]) % D) / D
        re, im = np.cos(ang), -np.sin(ang)
        if par == 0:
            im[0] = np.where(d % 2 == 0, 1.0, -1.0)
        blocks += [re, im]
    fd = np.concatenate(blocks, axis=0)
    n2 = np.arange(S // _R, dtype=np.int64)
    g = np.zeros((_R, 2 * (S // _R), 2 * (S // _R)))
    for n1 in range(_R):
        a = 2.0 * np.pi * (((n1 + _R * n2)[:, None] * n2[None, :]) % S) / S
        gr, gi = np.cos(a), -np.sin(a)
        g[n1] = np.block([[gr, gi], [-gi, gr]])
    g = g * np.sqrt(2.0 / (S * D))
    cast = lambda a: np.asarray(a, np.float32).astype(_BF16)
    g = g.reshape(_R, 2 * n2.size, 2, n2.size).transpose(0, 2, 1, 3)
    return cast(fd), cast(g)


def _cmul_const(z, j, n, sgn):
    re, im = z
    j %= n
    if j == 0:
        return re, im
    if 2 * j == n:
        return -re, -im
    if 4 * j == n:
        return (-im, re) if sgn > 0 else (im, -re)
    if 4 * j == 3 * n:
        return (im, -re) if sgn > 0 else (-im, re)
    c = float(np.cos(2 * np.pi * j / n))
    s = float(sgn * np.sin(2 * np.pi * j / n))
    if 8 * j % n == 0:
        a = re + im if c * s < 0 else re - im
        b = im - re if c * s < 0 else im + re
        return a * c, b * c
    return re * c - im * s, re * s + im * c


def _fft(zs, sgn):
    n = len(zs)
    if n == 1:
        return zs
    ev = _fft(zs[0::2], sgn)
    od = _fft(zs[1::2], sgn)
    out = [None] * n
    for j in range(n // 2):
        if 4 * j == n:
            (er, ei), (orr, oi) = ev[j], od[j]
            if sgn > 0:
                out[j], out[j + n // 2] = (er - oi, ei + orr), (er + oi, ei - orr)
            else:
                out[j], out[j + n // 2] = (er + oi, ei - orr), (er - oi, ei + orr)
            continue
        tr, ti = _cmul_const(od[j], j, n, sgn)
        out[j] = (ev[j][0] + tr, ev[j][1] + ti)
        out[j + n // 2] = (ev[j][0] - tr, ev[j][1] - ti)
    return out


def _halves(u):
    return (pltpu.bitcast(u << 16, _F32), pltpu.bitcast(u & jnp.uint32(0xFFFF0000), _F32))


def _kernel(ax_hbm, mem0_ref, wq_hbm, wk_hbm, wv_hbm, wo_hbm, bx_hbm, wr_hbm, wi_hbm,
            wrn_ref, win_ref, fd_hbm, g_hbm, out_hbm,
            ax, xtail, pre, stage, wqkv, wo, hbuf, obuf, acc, aout,
            bx, wr, wi, fd, g, ze, zo,
            sem_in, sem_x, sem_g, sem_w, sem_wo, sem_ao, sem_bo, *, S, D, H, M, seg):
    half, quart = D // 2, D // 4
    N2 = S // _R
    L = M + seg
    npair = H // 2
    w_hbms = (wq_hbm, wk_hbm, wv_hbm)
    nt = (((1,), (1,)), ((), ()))
    tn = (((0,), (0,)), ((), ()))

    in_copies = [
        pltpu.make_async_copy(fd_hbm, fd, sem_in.at[0]),
        None,
        pltpu.make_async_copy(wr_hbm.at[0:half].bitcast(_U32), wr, sem_in.at[2]),
        pltpu.make_async_copy(wi_hbm.at[0:half].bitcast(_U32), wi, sem_in.at[3]),
        pltpu.make_async_copy(ax_hbm.at[0:8], ax.at[0:8], sem_in.at[4]),
        pltpu.make_async_copy(ax_hbm.at[8:S // seg], ax.at[8:S // seg], sem_in.at[5]),
        pltpu.make_async_copy(ax_hbm.at[:, seg - 8:seg], xtail, sem_in.at[6]),
    ]
    G = 4
    ngroup = H // G

    def wo_copy(gi):
        rows = pl.ds(pl.multiple_of(gi * G * 64, G * 64), G * 64)
        return pltpu.make_async_copy(wo_hbm.bitcast(_U32).at[rows], wo.at[rows], sem_wo.at[gi])

    def bo_copy(a):
        return pltpu.make_async_copy(bx.at[a], out_hbm.bitcast(_U32).at[:, a, D:2 * D], sem_bo)

    def x_copy(a):
        return pltpu.make_async_copy(bx_hbm.bitcast(_U32).at[:, a, :], bx.at[a], sem_x.at[a])

    def w_copy(m, j):
        return pltpu.make_async_copy(w_hbms[m].bitcast(_U32).at[:, j, :],
                                     stage.at[m * npair + j], sem_w.at[m * npair + j])

    def g_copy(a):
        return pltpu.make_async_copy(g_hbm.at[pl.ds(2 * a, 2)], g.at[pl.ds(2 * a, 2)], sem_g.at[a])

    x_copy(0).start()
    in_copies[0].start()
    g_copy(0).start()
    for a in range(1, _R // 2):
        x_copy(a).start()
        g_copy(a).start()
    in_copies[0].wait()
    for i in (2, 3, 4):
        in_copies[i].start()
    for gi in range(ngroup):
        for j in range(gi * G // 2, (gi + 1) * G // 2):
            for m in range(3):
                w_copy(m, j).start()
        wo_copy(gi).start()
        if gi == 0:
            in_copies[6].start()

    first = jax.lax.broadcasted_iota(jnp.int32, (8, N2), 0) == 0
    lane0 = jax.lax.broadcasted_iota(jnp.int32, (N2, N2), 1) == 0

    def gmat(n1):
        return jnp.concatenate([g[n1, 0], g[n1, 1]], axis=1)

    def fwd_s(n1, zt):
        return jnp.dot(zt, gmat(n1), preferred_element_type=_F32)

    def inv_s(gm, yt):
        return jax.lax.dot_general(gm, yt, nt, preferred_element_type=_F32)

    def filt(zr, rows, ws):
        xs = _fft([(zr[n, rows, 0:N2], zr[n, rows, N2:2 * N2]) for n in range(_R)], -1)
        ys = [(xr * fr - xi * fi, xr * fi + xi * fr) for (xr, xi), (fr, fi) in zip(xs, ws)]
        for n, (yr, yi) in enumerate(_fft(ys, +1)):
            zr[n, rows, 0:N2] = yr
            zr[n, rows, N2:2 * N2] = yi

    def filt_rows(zr, par, j):
        rows = pl.ds(pl.multiple_of(j * 8, 8), 8)
        ws = [[_halves(ref[rows, l1 * N2:(l1 + 1) * N2])[par] for ref in (wr, wi)]
              for l1 in range(_R)]
        if par == 0:
            dc = jnp.where(first & (j == 0), 0.5, 1.0)
            ws = [[w * dc for w in f] for f in ws]
        filt(zr, rows, ws)

    def fwd_d(a, _):
        x_copy(a).wait()
        g_copy(a).wait()
        for b, x in enumerate(_halves(bx[a])):
            n1 = 2 * a + b
            xe, xo = x[:, 0:half] + x[:, half:D], x[:, 0:half] - x[:, half:D]
            ye = jax.lax.dot_general(fd[0:half, :], xe.astype(_BF16), nt,
                                     preferred_element_type=_F32)
            yo = jax.lax.dot_general(fd[half:D, :], xo.astype(_BF16), nt,
                                     preferred_element_type=_F32)
            top = ye[quart:quart + 8]
            re = jnp.concatenate([ye[0:quart], jnp.where(first, top, 0.0)], axis=0)
            im = jnp.concatenate([jnp.where(first, 0.0, top), ye[quart + 8:half],
                                  jnp.zeros((8, N2), _F32)], axis=0)
            ze[n1] = fwd_s(n1, jnp.concatenate([re, im], axis=1))
            zo[n1, :, 0:N2] = yo[0:quart]
            zo[n1, :, N2:2 * N2] = yo[quart:half]
        return 0
    jax.lax.fori_loop(0, _R // 2, fwd_d, 0)

    in_copies[2].wait()
    in_copies[3].wait()
    filt(ze, slice(quart, quart + 8),
         [[jnp.where(first, ref[0:8, l1 * N2:(l1 + 1) * N2].astype(_F32) * 0.5, 0.0)
           for ref in (wrn_ref, win_ref)] for l1 in range(_R)])
    per = quart // 8 // _R

    def mid_e(i, _):
        for n1 in (2 * i, 2 * i + 1):
            zo[n1] = fwd_s(n1, zo[n1])
            for t in range(per):
                filt_rows(ze, 0, n1 * per + t)
        return 0
    jax.lax.fori_loop(0, _R // 2, mid_e, 0)

    def mid_o(i, _):
        for n1 in (2 * i, 2 * i + 1):
            ze[n1, 0:quart, :] = inv_s(gmat(n1), ze[n1, 0:quart, :])
            for t in range(per):
                filt_rows(zo, 1, n1 * per + t)
        return 0
    jax.lax.fori_loop(0, _R // 2, mid_o, 0)

    def inv_d(a, _):
        ys = []
        for b in range(2):
            n1 = 2 * a + b
            gm = gmat(n1)
            un = inv_s(gm[0:N2], jnp.concatenate(
                [ze[n1, quart:quart + 8, :], jnp.zeros((N2 - 8, 2 * N2), _F32)], axis=0))
            uo = inv_s(gm, zo[n1])
            ue = jnp.concatenate([ze[n1, 0:N2, :], jnp.where(lane0, un, ze[n1, N2:2 * N2, 0:N2]),
                                  ze[n1, N2:2 * N2, N2:quart]], axis=1)
            p = jnp.dot(ue, fd[0:half, :], preferred_element_type=_F32)
            q = jnp.dot(jnp.concatenate([uo[0:N2], uo[N2:2 * N2]], axis=1), fd[half:D, :],
                        preferred_element_type=_F32)
            ys.append(jnp.concatenate([p + q, p - q], axis=1))
        bx[a] = pltpu.bitcast(pltpu.pack_elementwise(ys, packed_dtype=_BF16), _U32)
        return 0
    jax.lax.fori_loop(0, _R // 2, inv_d, 0)

    in_copies[4].wait()
    hbuf[0:M, :] = mem0_ref[...].astype(_F32)
    hbuf[M:L, :] = ax[0].astype(_F32)
    nseg = S // seg
    scale = float(np.asarray(128.0 ** -0.5, np.float32).astype(_BF16).astype(np.float32))
    neg = float(np.asarray(-1e9, np.float32).astype(_BF16).astype(np.float32))

    row = jax.lax.broadcasted_iota(jnp.int32, (L, 128), 0)
    col = jax.lax.broadcasted_iota(jnp.int32, (L, 128), 1)
    allowed = (col < L) & ((row < M) | (row >= col))
    fill = jnp.where(col < L, jnp.float32(neg), jnp.float32(-np.inf))

    def unit(m, h):
        return (h // G) * 3 + (1, 0, 2)[m]

    def weights(m, heads):
        return pltpu.bitcast(jnp.concatenate([wqkv[m, h] for h in heads], axis=1), _BF16)

    def proj(m, heads, s=None):
        if s is None or unit(m, heads[0]) >= _NPRE:
            y = jnp.dot(hbuf[...], weights(m, heads), preferred_element_type=_F32)
            return [y[:, i * 128:(i + 1) * 128] for i in range(len(heads))]
        y = jnp.dot(hbuf[0:L - 8, :], weights(m, heads), preferred_element_type=_F32)
        rows = pl.ds(pl.multiple_of(s * 8, 8), 8)
        return [jnp.concatenate([y[:, i * 128:(i + 1) * 128], pre[unit(m, h), h % G, rows, :]], axis=0)
                for i, h in enumerate(heads)]

    def pad_keys(t):
        return jnp.concatenate([t, jnp.zeros((128 - L, 128), _F32)], axis=0).astype(_BF16)

    def probs(q, k):
        s = jax.lax.dot_general(q, pad_keys(k), (((1,), (1,)), ((), ())),
                                preferred_element_type=_F32)
        s = jnp.where(allowed, s * scale, fill)
        e = jnp.exp(s - jnp.max(s, axis=1, keepdims=True))
        den = jnp.sum(e, axis=1, keepdims=True)
        r = pl.reciprocal(den, approx=True)
        return e * (r * (2.0 - den * r))

    def out_part(gi, n0, n1):
        c0, c1 = gi * G * 128, (gi + 1) * G * 128
        w = pltpu.bitcast(wo[c0 // 2:c1 // 2, n0:n1], _BF16)
        y = jnp.dot(obuf[:, c0:c1], w, preferred_element_type=_F32)
        if gi == 0:
            acc[:, n0:n1] = y
        else:
            acc[:, n0:n1] += y

    def values(heads, ps, vs):
        for h, p, v in zip(heads, ps, vs):
            obuf[:, h * 128:(h + 1) * 128] = jnp.dot(p, pad_keys(v), preferred_element_type=_F32)

    def group(s, gi, late):
        heads = list(range(gi * G, (gi + 1) * G))
        ks = proj(1, heads, s)
        if late is not None:
            values(*late)
        qs = proj(0, heads, s)
        vs = proj(2, heads[:2], s)
        ps = [probs(q, k) for q, k in zip(qs, ks)]
        vs += proj(2, heads[2:], s)
        if gi == 0:
            return heads, ps, vs
        out_part(gi - 1, 0, 768)
        values(heads, ps, vs)
        out_part(gi - 1, 768, D)

    def ao_copy(s):
        nb = seg // _R
        return pltpu.make_async_copy(aout.at[pl.ds(s * nb, nb)],
                                     out_hbm.at[pl.ds(s * nb, nb), :, 0:D], sem_ao)

    def finish(s):
        hbuf[0:M, :] = acc[0:M, :]
        nb = seg // _R
        for i in range(nb):
            aout[s * nb + i] = acc[M + i * _R:M + (i + 1) * _R, :].astype(_BF16)

    acc[...] = jnp.zeros((L, D), _F32)

    def first_group(gi, _):
        for jj in range(G // 2):
            j = gi * (G // 2) + jj
            for m in range(3):
                w_copy(m, j).wait()
                ev = stage[m * npair + j, pl.ds(0, half, stride=2), :]
                od = stage[m * npair + j, pl.ds(1, half, stride=2), :]
                wqkv[m, 2 * j] = (ev & jnp.uint32(0xFFFF)) | (od << 16)
                wqkv[m, 2 * j + 1] = (ev >> 16) | (od & jnp.uint32(0xFFFF0000))
        heads = [gi * G + i for i in range(G)]
        ks, qs, vs = proj(1, heads), proj(0, heads), proj(2, heads)
        o = jnp.concatenate([jnp.dot(probs(q, k), pad_keys(v), preferred_element_type=_F32)
                             for q, k, v in zip(qs, ks, vs)], axis=1)
        wo_copy(gi).wait()
        rows = pl.ds(pl.multiple_of(gi * G * 64, G * 64), G * 64)
        acc[...] += jnp.dot(o, pltpu.bitcast(wo[rows, :], _BF16), preferred_element_type=_F32)
        return 0
    npg = -(-_NPRE // 3)
    jax.lax.fori_loop(0, npg, first_group, 0)

    in_copies[6].wait()
    for u in range(_NPRE):
        m, gi = (1, 0, 2)[u % 3], u // 3

        def ahead(i, _, m=m, gi=gi, u=u):
            xt = xtail[...].astype(_F32).reshape(nseg * 8, D)
            heads = [gi * G + 2 * i, gi * G + 2 * i + 1]
            y = jnp.dot(xt, weights(m, heads), preferred_element_type=_F32)
            pre[u, 2 * i] = y[:, 0:128]
            pre[u, 2 * i + 1] = y[:, 128:256]
            return 0
        jax.lax.fori_loop(0, G // 2, ahead, 0)
    jax.lax.fori_loop(npg, ngroup, first_group, 0)
    in_copies[5].start()
    for a in range(_R // 2):
        bo_copy(a).start()
    hbuf[M:L, :] = ax[1].astype(_F32)
    finish(0)

    def step(s, _):
        @pl.when(s == 7)
        def _():
            in_copies[5].wait()
        late = None
        for gi in range(ngroup):
            late = group(s, gi, late)
            if gi == 0:
                ao_copy(s - 1).start()
        hbuf[M:L, :] = ax[jnp.minimum(s + 1, nseg - 1)].astype(_F32)
        out_part(ngroup - 1, 0, D)
        finish(s)
        return 0
    jax.lax.fori_loop(1, nseg, step, 0)
    ao_copy(nseg - 1).start()

    pltpu.make_async_copy(aout, out_hbm.at[:, :, 0:D], sem_ao).wait()
    for a in range(_R // 2):
        bo_copy(a).wait()


@functools.partial(jax.jit, static_argnames=("A_seg_len",))
def pallas_concat_heads__memory_aug_recurrent_mem_tr__spectral_gfnet__prompt_kernel(
    A_x, A_mem0, A_Wq, A_Wk, A_Wv, A_Wo, A_seg_len, B_x, B_w_r, B_w_i,
):
    _, S, D = A_x.shape
    H, Dh = A_Wq.shape[1], A_Wq.shape[2]
    M = A_mem0.shape[1]
    seg = int(A_seg_len)
    assert (S, D, H, Dh, M, seg) == (2048, 1024, 32, 128, 8, 32) and B_x.shape == (1, S, D)
    L = M + seg
    half = D // 2
    N2 = S // _R
    fd, g = _dft_constants(S, D)
    wr_t, wi_t = B_w_r.T, B_w_i.T
    nyq = pl.BlockSpec((16, S), lambda i: (half // 16, 0))

    hbm = pl.BlockSpec(memory_space=pl.ANY)
    vm = pltpu.VMEM
    out = pl.pallas_call(
        functools.partial(_kernel, S=S, D=D, H=H, M=M, seg=seg),
        out_shape=jax.ShapeDtypeStruct((N2, _R, 2 * D), _BF16),
        grid=(1,),
        in_specs=[hbm, pl.BlockSpec(memory_space=pltpu.VMEM)] + [hbm] * 7 + [nyq, nyq, hbm, hbm],
        out_specs=hbm,
        scratch_shapes=[
            vm((S // seg, seg, D), _BF16),
            vm((S // seg, 8, D), _BF16),
            vm((max(_NPRE, 1), 4, S // seg * 8, Dh), _F32),
            vm((3 * H // 2, D, Dh), _U32),
            vm((3, H, D // 2, Dh), _U32),
            vm((H * Dh // 2, D), _U32),
            vm((L, D), _F32),
            vm((L, H * Dh), _F32),
            vm((L, D), _F32),
            vm((N2, _R, D), _BF16),
            vm((_R // 2, N2, D), _U32),
            vm((half // 2, S), _U32),
            vm((half // 2, S), _U32),
            vm((D, half), _BF16),
            vm((_R, 2, 2 * N2, N2), _BF16),
            vm((_R, half // 2 + 8, 2 * N2), _F32),
            vm((_R, half // 2, 2 * N2), _F32),
            pltpu.SemaphoreType.DMA((7,)),
            pltpu.SemaphoreType.DMA((_R // 2,)),
            pltpu.SemaphoreType.DMA((_R // 2,)),
            pltpu.SemaphoreType.DMA((3 * H // 2,)),
            pltpu.SemaphoreType.DMA((H // 4,)),
            pltpu.SemaphoreType.DMA,
            pltpu.SemaphoreType.DMA,
        ],
        compiler_params=pltpu.CompilerParams(vmem_limit_bytes=120 * 1024 * 1024),
    )(A_x.reshape(S // seg, seg, D), A_mem0.reshape(M, D), A_Wq, A_Wk, A_Wv, A_Wo.reshape(H * Dh, D),
      B_x.reshape(N2, _R, D), wr_t, wi_t, wr_t, wi_t, fd, g)
    return out.reshape(1, S, 2 * D)
```

```python
import functools

import jax
import jax.numpy as jnp
import numpy as np
import jax.experimental.pallas as pl
import jax.experimental.pallas.tpu as pltpu

_F32 = jnp.float32
_BF16 = jnp.bfloat16
_U32 = jnp.uint32

_R = 16
_NPRE = 6
_SQ = float(np.sqrt(0.5))


def _dft_constants(S, D):
    half, quart = D // 2, D // 4
    m = np.arange(D // 8, dtype=np.int64)

    def block(k, n):
        ang = 2.0 * np.pi * ((k[:, None] * np.arange(n, dtype=np.int64)[None, :]) % D) / D
        return np.concatenate([np.cos(ang), -np.sin(ang)], axis=0)

    fo = block(np.concatenate([4 * m + 1, 4 * m + 3]), half)
    f2 = block(4 * m + 2, quart)
    f0 = block(4 * m, quart)
    f0[m.size] = np.where(np.arange(quart) % 2 == 0, 1.0, -1.0)
    fe = np.concatenate([f0, f2], axis=0)
    n2 = np.arange(S // _R, dtype=np.int64)
    g = np.zeros((_R, 2 * (S // _R), 2 * (S // _R)))
    for n1 in range(_R):
        a = 2.0 * np.pi * (((n1 + _R * n2)[:, None] * n2[None, :]) % S) / S
        gr, gi = np.cos(a), -np.sin(a)
        g[n1] = np.block([[gr, gi], [-gi, gr]])
    g = g * np.sqrt(2.0 / (S * D))
    cast = lambda a: np.asarray(a, np.float32).astype(_BF16)
    g = g.reshape(_R, 2 * n2.size, 2, n2.size).transpose(0, 2, 1, 3)
    return cast(fo), cast(fe), cast(g)


def _cmul_const(z, j, n, sgn):
    re, im = z
    j %= n
    if j == 0:
        return re, im
    if 2 * j == n:
        return -re, -im
    if 4 * j == n:
        return (-im, re) if sgn > 0 else (im, -re)
    if 4 * j == 3 * n:
        return (im, -re) if sgn > 0 else (-im, re)
    c = float(np.cos(2 * np.pi * j / n))
    s = float(sgn * np.sin(2 * np.pi * j / n))
    if 8 * j % n == 0:
        a = re + im if c * s < 0 else re - im
        b = im - re if c * s < 0 else im + re
        return a * c, b * c
    return re * c - im * s, re * s + im * c


def _fft(zs, sgn):
    n = len(zs)
    if n == 1:
        return zs
    ev = _fft(zs[0::2], sgn)
    od = _fft(zs[1::2], sgn)
    out = [None] * n
    for j in range(n // 2):
        if 4 * j == n:
            (er, ei), (orr, oi) = ev[j], od[j]
            if sgn > 0:
                out[j], out[j + n // 2] = (er - oi, ei + orr), (er + oi, ei - orr)
            else:
                out[j], out[j + n // 2] = (er + oi, ei - orr), (er - oi, ei + orr)
            continue
        tr, ti = _cmul_const(od[j], j, n, sgn)
        out[j] = (ev[j][0] + tr, ev[j][1] + ti)
        out[j + n // 2] = (ev[j][0] - tr, ev[j][1] - ti)
    return out


def _halves(u):
    return (pltpu.bitcast(u << 16, _F32), pltpu.bitcast(u & jnp.uint32(0xFFFF0000), _F32))


def _kernel(ax_hbm, mem0_ref, wq_hbm, wk_hbm, wv_hbm, wo_hbm, bx_hbm, wr_hbm, wi_hbm,
            wrn_ref, win_ref, fo_hbm, fe_hbm, g_hbm, out_hbm,
            ax, xtail, pre, stage, wqkv, wo, hbuf, obuf, acc, aout,
            bx, wr, wi, fo, fe, g, ze, zo,
            sem_in, sem_x, sem_g, sem_w, sem_wo, sem_ao, sem_bo, *, S, D, H, M, seg):
    half, quart, eight = D // 2, D // 4, D // 8
    N2 = S // _R
    L = M + seg
    npair = H // 2
    w_hbms = (wq_hbm, wk_hbm, wv_hbm)
    nt = (((1,), (1,)), ((), ()))
    tn = (((0,), (0,)), ((), ()))

    in_copies = [
        pltpu.make_async_copy(fo_hbm, fo, sem_in.at[0]),
        pltpu.make_async_copy(fe_hbm, fe, sem_in.at[1]),
        None,
        None,
        pltpu.make_async_copy(ax_hbm.at[0:8], ax.at[0:8], sem_in.at[4]),
        pltpu.make_async_copy(ax_hbm.at[8:S // seg], ax.at[8:S // seg], sem_in.at[5]),
        pltpu.make_async_copy(ax_hbm.at[:, seg - 8:seg], xtail, sem_in.at[6]),
    ]
    G = 4
    ngroup = H // G

    def wo_copy(gi):
        rows = pl.ds(pl.multiple_of(gi * G * 64, G * 64), G * 64)
        return pltpu.make_async_copy(wo_hbm.bitcast(_U32).at[rows], wo.at[rows], sem_wo.at[gi])

    def bo_copy(a):
        return pltpu.make_async_copy(bx.at[a], out_hbm.bitcast(_U32).at[:, a, D:2 * D], sem_bo)

    def x_copy(a):
        return pltpu.make_async_copy(bx_hbm.bitcast(_U32).at[:, a, :], bx.at[a], sem_x.at[a])

    def w_copy(m, j):
        return pltpu.make_async_copy(w_hbms[m].bitcast(_U32).at[:, j, :],
                                     stage.at[3 * j + m], sem_w.at[3 * j + m])

    def arrived(p):
        pltpu.make_async_copy(stage.at[p], stage.at[p], sem_w.at[p]).wait()

    def relayout(p0, n):
        words = [[stage[p0 + i, pl.ds(r, half, stride=2), :] for r in range(2)] for i in range(n)]
        for i, (ev, od) in enumerate(words):
            j, m = (p0 + i) // 3, (p0 + i) % 3
            wqkv[m, 2 * j] = (ev & jnp.uint32(0xFFFF)) | (od << 16)
            wqkv[m, 2 * j + 1] = (ev >> 16) | (od & jnp.uint32(0xFFFF0000))

    def g_copy(a):
        return pltpu.make_async_copy(g_hbm.at[pl.ds(2 * a, 2)], g.at[pl.ds(2 * a, 2)], sem_g.at[a])

    x_copy(0).start()
    in_copies[0].start()
    in_copies[1].start()
    g_copy(0).start()
    for a in range(1, _R // 2):
        x_copy(a).start()
        g_copy(a).start()
    in_copies[0].wait()
    in_copies[1].wait()
    f_copies = [
        pltpu.make_async_copy(src.at[0:half].bitcast(_U32).at[:, l1 * N2:(l1 + 1) * N2],
                              dst.at[l1], sem_in.at[2])
        for src, dst in ((wr_hbm, wr), (wi_hbm, wi)) for l1 in range(_R)]
    for c in f_copies + [in_copies[4], in_copies[6]]:
        c.start()

    first = jax.lax.broadcasted_iota(jnp.int32, (8, N2), 0) == 0
    lane0 = jax.lax.broadcasted_iota(jnp.int32, (N2, N2), 1) == 0

    def gmat(n1):
        return jnp.concatenate([g[n1, 0], g[n1, 1]], axis=1)

    def fwd_s(n1, zt):
        return jnp.dot(zt, gmat(n1), preferred_element_type=_F32)

    def inv_s(gm, yt):
        return jax.lax.dot_general(gm, yt, nt, preferred_element_type=_F32)

    def filt(zr, rows, ws):
        xs = _fft([(zr[n, rows, 0:N2], zr[n, rows, N2:2 * N2]) for n in range(_R)], -1)
        ys = [(xr * fr - xi * fi, xr * fi + xi * fr) for (xr, xi), (fr, fi) in zip(xs, ws)]
        for n, (yr, yi) in enumerate(_fft(ys, +1)):
            zr[n, rows, 0:N2] = yr
            zr[n, rows, N2:2 * N2] = yi

    def filt_rows(zr, par, c, j):
        rows = pl.ds(pl.multiple_of(c * eight + j * 8, 8), 8)
        ws = [[_halves(ref[l1, pl.ds(16 * j + c, 8, stride=2), :])[par] for ref in (wr, wi)]
              for l1 in range(_R)]
        if par == 0 and c == 0:
            dc = jnp.where(first & (j == 0), 0.5, 1.0)
            ws = [[w * dc for w in f] for f in ws]
        filt(zr, rows, ws)

    assert ngroup == _R // 2

    def fwd_d(a, _):
        for j in range(G // 2):
            for m in range(3):
                w_copy(m, a * (G // 2) + j).start()
        wo_copy(a).start()
        x_copy(a).wait()
        g_copy(a).wait()
        for b, x in enumerate(_halves(bx[a])):
            n1 = 2 * a + b
            xe, xo = x[:, 0:half] + x[:, half:D], x[:, 0:half] - x[:, half:D]
            x0, x2 = xe[:, 0:quart] + xe[:, quart:half], xe[:, 0:quart] - xe[:, quart:half]
            y0 = jax.lax.dot_general(fe[0:quart, :], x0.astype(_BF16), nt,
                                     preferred_element_type=_F32)
            y2 = jax.lax.dot_general(fe[quart:half, :], x2.astype(_BF16), nt,
                                     preferred_element_type=_F32)
            yo = jax.lax.dot_general(fo[...], xo.astype(_BF16), nt, preferred_element_type=_F32)
            top = y0[eight:eight + 8]
            re = jnp.concatenate([y0[0:eight], y2[0:eight], jnp.where(first, top, 0.0)], axis=0)
            im = jnp.concatenate([jnp.where(first, 0.0, top), y0[eight + 8:quart], y2[eight:quart],
                                  jnp.zeros((8, N2), _F32)], axis=0)
            ze[n1] = fwd_s(n1, jnp.concatenate([re, im], axis=1))
            zo[n1, :, 0:N2] = yo[0:quart]
            zo[n1, :, N2:2 * N2] = yo[quart:half]
        return 0
    jax.lax.fori_loop(0, _R // 2, fwd_d, 0)

    for c in f_copies:
        c.wait()
    filt(ze, slice(quart, quart + 8),
         [[jnp.where(first, ref[0:8, l1 * N2:(l1 + 1) * N2].astype(_F32) * 0.5, 0.0)
           for ref in (wrn_ref, win_ref)] for l1 in range(_R)])
    assert eight // 8 == _R

    def mid_e(i, _):
        for n1 in (2 * i, 2 * i + 1):
            zo[n1] = fwd_s(n1, zo[n1])
            for c in range(2):
                filt_rows(ze, 0, c, n1)
        return 0
    jax.lax.fori_loop(0, _R // 2, mid_e, 0)

    def mid_o(i, _):
        for n1 in (2 * i, 2 * i + 1):
            ze[n1, 0:quart, :] = inv_s(gmat(n1), ze[n1, 0:quart, :])
            for c in range(2):
                filt_rows(zo, 1, c, n1)
        return 0
    jax.lax.fori_loop(0, _R // 2, mid_o, 0)

    def inv_d(a, _):
        arrived(2 * a)
        arrived(2 * a + 1)
        ys = []
        for b in range(2):
            n1 = 2 * a + b
            gm = gmat(n1)
            un = inv_s(gm[0:N2], jnp.concatenate(
                [ze[n1, quart:quart + 8, :], jnp.zeros((N2 - 8, 2 * N2), _F32)], axis=0))
            uo = inv_s(gm, zo[n1])
            u0 = jnp.concatenate([ze[n1, 0:N2, 0:eight],
                                  jnp.where(lane0, un, ze[n1, N2:2 * N2, 0:eight])], axis=1)
            u2 = jnp.concatenate([ze[n1, 0:N2, eight:quart], ze[n1, N2:2 * N2, eight:quart]], axis=1)
            p2 = jnp.dot(u2, fe[quart:half, :], preferred_element_type=_F32)
            p0 = jnp.dot(u0, fe[0:quart, :], preferred_element_type=_F32)
            p = jnp.concatenate([p0 + p2, p0 - p2], axis=1)
            q = jnp.dot(jnp.concatenate([uo[0:N2], uo[N2:2 * N2]], axis=1), fo[...],
                        preferred_element_type=_F32)
            ys.append(jnp.concatenate([p + q, p - q], axis=1))
        relayout(2 * a, 2)
        bx[a] = pltpu.bitcast(pltpu.pack_elementwise(ys, packed_dtype=_BF16), _U32)
        return 0
    jax.lax.fori_loop(0, _R // 2, inv_d, 0)

    in_copies[4].wait()
    hbuf[0:M, :] = mem0_ref[...].astype(_F32)
    hbuf[M:L, :] = ax[0].astype(_F32)
    nseg = S // seg
    scale = float(np.asarray(128.0 ** -0.5, np.float32).astype(_BF16).astype(np.float32))
    neg = float(np.asarray(-1e9, np.float32).astype(_BF16).astype(np.float32))

    row = jax.lax.broadcasted_iota(jnp.int32, (L, 128), 0)
    col = jax.lax.broadcasted_iota(jnp.int32, (L, 128), 1)
    allowed = (col < L) & ((row < M) | (row >= col))
    fill = jnp.where(col < L, jnp.float32(neg), jnp.float32(-np.inf))

    def unit(m, h):
        return (h // G) * 3 + (1, 0, 2)[m]

    def weights(m, heads):
        return pltpu.bitcast(jnp.concatenate([wqkv[m, h] for h in heads], axis=1), _BF16)

    def proj(m, heads, s=None, mem=None):
        rows_to = lambda n: (hbuf[0:n, :] if mem is None else jnp.concatenate([mem, hbuf[M:n, :]], axis=0))
        if s is None or unit(m, heads[0]) >= _NPRE:
            y = jnp.dot(rows_to(L), weights(m, heads), preferred_element_type=_F32)
            return [y[:, i * 128:(i + 1) * 128] for i in range(len(heads))]
        y = jnp.dot(rows_to(L - 8), weights(m, heads), preferred_element_type=_F32)
        rows = pl.ds(pl.multiple_of(s * 8, 8), 8)
        return [jnp.concatenate([y[:, i * 128:(i + 1) * 128], pre[unit(m, h), h % G, rows, :]], axis=0)
                for i, h in enumerate(heads)]

    def pad_keys(t):
        return jnp.concatenate([t, jnp.zeros((128 - L, 128), _F32)], axis=0).astype(_BF16)

    def probs(q, k):
        s = jax.lax.dot_general(q, pad_keys(k), (((1,), (1,)), ((), ())),
                                preferred_element_type=_F32)
        s = jnp.where(allowed, s * scale, fill)
        e = jnp.exp(s - jnp.max(s, axis=1, keepdims=True))
        den = jnp.sum(e, axis=1, keepdims=True)
        r = pl.reciprocal(den, approx=True)
        return e * (r * (2.0 - den * r))

    def out_part(gi, n0, n1):
        c0, c1 = gi * G * 128, (gi + 1) * G * 128
        w = pltpu.bitcast(wo[c0 // 2:c1 // 2, n0:n1], _BF16)
        y = jnp.dot(obuf[:, c0:c1], w, preferred_element_type=_F32)
        if gi == 0:
            acc[:, n0:n1] = y
        elif gi < ngroup - 1:
            acc[:, n0:n1] += y
        else:
            return acc[:, n0:n1] + y

    def values(heads, ps, vs):
        for h, p, v in zip(heads, ps, vs):
            obuf[:, h * 128:(h + 1) * 128] = jnp.dot(p, pad_keys(v), preferred_element_type=_F32)

    def group(s, gi, late, mem):
        heads = list(range(gi * G, (gi + 1) * G))
        ks = proj(1, heads, s, mem)
        if late is not None:
            values(*late)
        qs = proj(0, heads, s, mem)
        vs = proj(2, heads[:2], s, mem)
        ps = [probs(q, k) for q, k in zip(qs, ks)]
        vs += proj(2, heads[2:], s, mem)
        if gi == 0:
            return heads, ps, vs
        out_part(gi - 1, 0, 768)
        values(heads, ps, vs)
        out_part(gi - 1, 768, D)

    def ao_copy(s):
        nb = seg // _R
        return pltpu.make_async_copy(aout.at[pl.ds(s * nb, nb)],
                                     out_hbm.at[pl.ds(s * nb, nb), :, 0:D], sem_ao)

    def emit(s):
        nb = seg // _R
        for i in range(nb):
            aout[s * nb + i] = acc[M + i * _R:M + (i + 1) * _R, :].astype(_BF16)
        ao_copy(s).start()


    def first_group(todo, gi, _):
        for p in range(todo):
            arrived(6 * gi + 6 - todo + p)
            relayout(6 * gi + 6 - todo + p, 1)
        heads = [gi * G + i for i in range(G)]
        ks, qs, vs = proj(1, heads), proj(0, heads), proj(2, heads)
        o = jnp.concatenate([jnp.dot(probs(q, k), pad_keys(v), preferred_element_type=_F32)
                             for q, k, v in zip(qs, ks, vs)], axis=1)
        wo_copy(gi).wait()
        rows = pl.ds(pl.multiple_of(gi * G * 64, G * 64), G * 64)
        acc[...] += jnp.dot(o, pltpu.bitcast(wo[rows, :], _BF16), preferred_element_type=_F32)
        return 0
    in_copies[6].wait()
    for u in range(_NPRE):
        m, gi = (1, 0, 2)[u % 3], u // 3

        def ahead(i, _, m=m, gi=gi, u=u):
            arrived(_R + 4 * u + 2 * i)
            arrived(_R + 4 * u + 2 * i + 1)
            xt = xtail[...].astype(_F32).reshape(nseg * 8, D)
            heads = [gi * G + 2 * i, gi * G + 2 * i + 1]
            y = jnp.dot(xt, weights(m, heads), preferred_element_type=_F32)
            pre[u, 2 * i] = y[:, 0:128]
            pre[u, 2 * i + 1] = y[:, 128:256]
            relayout(_R + 4 * u + 2 * i, 1)
            relayout(_R + 4 * u + 2 * i + 1, 1)
            return 0
        jax.lax.fori_loop(0, G // 2, ahead, 0)
    done = _R + 4 * _NPRE
    assert 6 * -(-_NPRE // 3) <= _R and done < 6 * ngroup
    for gi in range(done // 6):
        wo_copy(gi).wait()
    late = None
    for gi in range(done // 6):
        late = group(None, gi, late, None)
    out_part(done // 6 - 1, 0, D)
    if done % 6:
        first_group(6 - done % 6, done // 6, 0)
    late_group = functools.partial(first_group, 6)
    jax.lax.fori_loop(-(-done // 6), ngroup, late_group, 0)
    in_copies[5].start()
    for a in range(_R // 2):
        bo_copy(a).start()
    hbuf[M:L, :] = ax[1].astype(_F32)

    def step(s, mem):
        late = None
        for gi in range(ngroup):
            late = group(s, gi, late, mem)
            if gi == 0:
                emit(s - 1)
        hbuf[M:L, :] = ax[jnp.minimum(s + 1, nseg - 1)].astype(_F32)
        y = out_part(ngroup - 1, 0, D)
        acc[M:L, :] = y[M:L]
        return y[0:M]
    mem = jax.lax.fori_loop(1, 4, step, acc[0:M, :])
    in_copies[5].wait()
    jax.lax.fori_loop(4, nseg, step, mem, unroll=2)
    emit(nseg - 1)

    pltpu.make_async_copy(aout, out_hbm.at[:, :, 0:D], sem_ao).wait()
    for a in range(_R // 2):
        bo_copy(a).wait()


@functools.partial(jax.jit, static_argnames=("A_seg_len",))
def pallas_concat_heads__memory_aug_recurrent_mem_tr__spectral_gfnet__prompt_kernel(
    A_x, A_mem0, A_Wq, A_Wk, A_Wv, A_Wo, A_seg_len, B_x, B_w_r, B_w_i,
):
    _, S, D = A_x.shape
    H, Dh = A_Wq.shape[1], A_Wq.shape[2]
    M = A_mem0.shape[1]
    seg = int(A_seg_len)
    assert (S, D, H, Dh, M, seg) == (2048, 1024, 32, 128, 8, 32) and B_x.shape == (1, S, D)
    L = M + seg
    half = D // 2
    N2 = S // _R
    fo, fe, g = _dft_constants(S, D)
    wr_t, wi_t = B_w_r.T, B_w_i.T
    nyq = pl.BlockSpec((16, S), lambda i: (half // 16, 0))

    hbm = pl.BlockSpec(memory_space=pl.ANY)
    vm = pltpu.VMEM
    out = pl.pallas_call(
        functools.partial(_kernel, S=S, D=D, H=H, M=M, seg=seg),
        out_shape=jax.ShapeDtypeStruct((N2, _R, 2 * D), _BF16),
        grid=(1,),
        in_specs=[hbm, pl.BlockSpec(memory_space=pltpu.VMEM)] + [hbm] * 7 + [nyq, nyq, hbm, hbm, hbm],
        out_specs=hbm,
        scratch_shapes=[
            vm((S // seg, seg, D), _BF16),
            vm((S // seg, 8, D), _BF16),
            vm((max(_NPRE, 1), 4, S // seg * 8, Dh), _F32),
            vm((3 * H // 2, D, Dh), _U32),
            vm((3, H, D // 2, Dh), _U32),
            vm((H * Dh // 2, D), _U32),
            vm((L, D), _F32),
            vm((L, H * Dh), _F32),
            vm((L, D), _F32),
            vm((N2, _R, D), _BF16),
            vm((_R // 2, N2, D), _U32),
            vm((_R, half // 2, N2), _U32),
            vm((_R, half // 2, N2), _U32),
            vm((half, half), _BF16),
            vm((half, half // 2), _BF16),
            vm((_R, 2, 2 * N2, N2), _BF16),
            vm((_R, half // 2 + 8, 2 * N2), _F32),
            vm((_R, half // 2, 2 * N2), _F32),
            pltpu.SemaphoreType.DMA((7,)),
            pltpu.SemaphoreType.DMA((_R // 2,)),
            pltpu.SemaphoreType.DMA((_R // 2,)),
            pltpu.SemaphoreType.DMA((3 * H // 2,)),
            pltpu.SemaphoreType.DMA((H // 4,)),
            pltpu.SemaphoreType.DMA,
            pltpu.SemaphoreType.DMA,
        ],
        compiler_params=pltpu.CompilerParams(vmem_limit_bytes=120 * 1024 * 1024),
    )(A_x.reshape(S // seg, seg, D), A_mem0.reshape(M, D), A_Wq, A_Wk, A_Wv, A_Wo.reshape(H * Dh, D),
      B_x.reshape(N2, _R, D), wr_t, wi_t, wr_t, wi_t, fo, fe, g)
    return out.reshape(1, S, 2 * D)
```

```python
import functools

import jax
import jax.numpy as jnp
import numpy as np
import jax.experimental.pallas as pl
import jax.experimental.pallas.tpu as pltpu

_F32 = jnp.float32
_BF16 = jnp.bfloat16
_U32 = jnp.uint32

_R = 16
_NPRE = 6
_SQ = float(np.sqrt(0.5))


def _dft_constants(S, D):
    half, quart = D // 2, D // 4
    m = np.arange(D // 8, dtype=np.int64)

    def block(k, n):
        ang = 2.0 * np.pi * ((k[:, None] * np.arange(n, dtype=np.int64)[None, :]) % D) / D
        return np.concatenate([np.cos(ang), -np.sin(ang)], axis=0)

    fo = block(np.concatenate([4 * m + 1, 4 * m + 3]), half)
    f2 = block(4 * m + 2, quart)
    f0 = block(4 * m, quart)
    f0[m.size] = np.where(np.arange(quart) % 2 == 0, 1.0, -1.0)
    fe = np.concatenate([f0, f2], axis=0)
    n2 = np.arange(S // _R, dtype=np.int64)
    g = np.zeros((_R, 2 * (S // _R), 2 * (S // _R)))
    for n1 in range(_R):
        a = 2.0 * np.pi * (((n1 + _R * n2)[:, None] * n2[None, :]) % S) / S
        gr, gi = np.cos(a), -np.sin(a)
        g[n1] = np.block([[gr, gi], [-gi, gr]])
    g = g * np.sqrt(2.0 / (S * D))
    cast = lambda a: np.asarray(a, np.float32).astype(_BF16)
    g = g.reshape(_R, 2 * n2.size, 2, n2.size).transpose(0, 2, 1, 3)
    return cast(fo), cast(fe), cast(g)


def _cmul_const(z, j, n, sgn):
    re, im = z
    j %= n
    if j == 0:
        return re, im
    if 2 * j == n:
        return -re, -im
    if 4 * j == n:
        return (-im, re) if sgn > 0 else (im, -re)
    if 4 * j == 3 * n:
        return (im, -re) if sgn > 0 else (-im, re)
    c = float(np.cos(2 * np.pi * j / n))
    s = float(sgn * np.sin(2 * np.pi * j / n))
    if 8 * j % n == 0:
        a = re + im if c * s < 0 else re - im
        b = im - re if c * s < 0 else im + re
        return a * c, b * c
    return re * c - im * s, re * s + im * c


def _fft(zs, sgn):
    n = len(zs)
    if n == 1:
        return zs
    ev = _fft(zs[0::2], sgn)
    od = _fft(zs[1::2], sgn)
    out = [None] * n
    for j in range(n // 2):
        if 4 * j == n:
            (er, ei), (orr, oi) = ev[j], od[j]
            if sgn > 0:
                out[j], out[j + n // 2] = (er - oi, ei + orr), (er + oi, ei - orr)
            else:
                out[j], out[j + n // 2] = (er + oi, ei - orr), (er - oi, ei + orr)
            continue
        tr, ti = _cmul_const(od[j], j, n, sgn)
        out[j] = (ev[j][0] + tr, ev[j][1] + ti)
        out[j + n // 2] = (ev[j][0] - tr, ev[j][1] - ti)
    return out


def _halves(u):
    return (pltpu.bitcast(u << 16, _F32), pltpu.bitcast(u & jnp.uint32(0xFFFF0000), _F32))


def _kernel(ax_hbm, mem0_ref, wq_hbm, wk_hbm, wv_hbm, wo_hbm, bx_hbm, wr_hbm, wi_hbm,
            wrn_ref, win_ref, fo_hbm, fe_hbm, g_hbm, out_hbm,
            ax, xtail, pre, stage, wqkv, wo, hbuf, obuf, acc, aout,
            bx, wr, wi, fo, fe, g, ze, zo,
            sem_in, sem_x, sem_g, sem_w, sem_wo, sem_ao, sem_bo, *, S, D, H, M, seg):
    half, quart, eight = D // 2, D // 4, D // 8
    N2 = S // _R
    L = M + seg
    npair = H // 2
    w_hbms = (wq_hbm, wk_hbm, wv_hbm)
    nt = (((1,), (1,)), ((), ()))
    tn = (((0,), (0,)), ((), ()))

    in_copies = [
        pltpu.make_async_copy(fo_hbm, fo, sem_in.at[0]),
        pltpu.make_async_copy(fe_hbm, fe, sem_in.at[1]),
        None,
        None,
        pltpu.make_async_copy(ax_hbm.at[0:8], ax.at[0:8], sem_in.at[4]),
        pltpu.make_async_copy(ax_hbm.at[8:S // seg], ax.at[8:S // seg], sem_in.at[5]),
        pltpu.make_async_copy(ax_hbm.at[:, seg - 8:seg], xtail, sem_in.at[6]),
    ]
    G = 4
    ngroup = H // G

    def wo_copy(gi):
        rows = pl.ds(pl.multiple_of(gi * G * 64, G * 64), G * 64)
        return pltpu.make_async_copy(wo_hbm.bitcast(_U32).at[rows], wo.at[rows], sem_wo.at[gi])

    def bo_copy(a):
        return pltpu.make_async_copy(bx.at[a], out_hbm.bitcast(_U32).at[:, a, D:2 * D], sem_bo)

    def x_copy(a):
        return pltpu.make_async_copy(bx_hbm.bitcast(_U32).at[:, a, :], bx.at[a], sem_x.at[a])

    def w_copy(m, j):
        return pltpu.make_async_copy(w_hbms[m].bitcast(_U32).at[:, j, :],
                                     stage.at[3 * j + m], sem_w.at[3 * j + m])

    def arrived(p):
        pltpu.make_async_copy(stage.at[p], stage.at[p], sem_w.at[p]).wait()

    def relayout(p0, n):
        words = [[stage[p0 + i, pl.ds(r, half, stride=2), :] for r in range(2)] for i in range(n)]
        for i, (ev, od) in enumerate(words):
            j, m = (p0 + i) // 3, (p0 + i) % 3
            wqkv[m, 2 * j] = (ev & jnp.uint32(0xFFFF)) | (od << 16)
            wqkv[m, 2 * j + 1] = (ev >> 16) | (od & jnp.uint32(0xFFFF0000))

    def g_copy(a):
        return pltpu.make_async_copy(g_hbm.at[pl.ds(2 * a, 2)], g.at[pl.ds(2 * a, 2)], sem_g.at[a])

    x_copy(0).start()
    in_copies[0].start()
    in_copies[1].start()
    g_copy(0).start()
    for a in range(1, _R // 2):
        x_copy(a).start()
        g_copy(a).start()
    in_copies[0].wait()
    in_copies[1].wait()
    f_copies = [
        pltpu.make_async_copy(src.at[0:half].bitcast(_U32).at[:, l1 * N2:(l1 + 1) * N2],
                              dst.at[l1], sem_in.at[2])
        for src, dst in ((wr_hbm, wr), (wi_hbm, wi)) for l1 in range(_R)]
    for c in f_copies + [in_copies[4], in_copies[6]]:
        c.start()

    first = jax.lax.broadcasted_iota(jnp.int32, (8, N2), 0) == 0
    lane0 = jax.lax.broadcasted_iota(jnp.int32, (N2, N2), 1) == 0

    def gmat(n1):
        return jnp.concatenate([g[n1, 0], g[n1, 1]], axis=1)

    def fwd_s(n1, zt):
        return jnp.dot(zt, gmat(n1), preferred_element_type=_F32)

    def inv_s(gm, yt):
        return jax.lax.dot_general(gm, yt, nt, preferred_element_type=_F32)

    def filt(zr, rows, ws):
        xs = _fft([(zr[n, rows, 0:N2], zr[n, rows, N2:2 * N2]) for n in range(_R)], -1)
        ys = [(xr * fr - xi * fi, xr * fi + xi * fr) for (xr, xi), (fr, fi) in zip(xs, ws)]
        for n, (yr, yi) in enumerate(_fft(ys, +1)):
            zr[n, rows, 0:N2] = yr
            zr[n, rows, N2:2 * N2] = yi

    def filt_rows(zr, par, c, j):
        rows = pl.ds(pl.multiple_of(c * eight + j * 8, 8), 8)
        ws = [[_halves(ref[l1, pl.ds(16 * j + c, 8, stride=2), :])[par] for ref in (wr, wi)]
              for l1 in range(_R)]
        if par == 0 and c == 0:
            dc = jnp.where(first & (j == 0), 0.5, 1.0)
            ws = [[w * dc for w in f] for f in ws]
        filt(zr, rows, ws)

    assert ngroup == _R // 2

    def fwd_d(a, _):
        for j in range(G // 2):
            for m in range(3):
                w_copy(m, a * (G // 2) + j).start()
        wo_copy(a).start()
        x_copy(a).wait()
        g_copy(a).wait()
        for b, x in enumerate(_halves(bx[a])):
            n1 = 2 * a + b
            xe, xo = x[:, 0:half] + x[:, half:D], x[:, 0:half] - x[:, half:D]
            x0, x2 = xe[:, 0:quart] + xe[:, quart:half], xe[:, 0:quart] - xe[:, quart:half]
            y0 = jax.lax.dot_general(fe[0:quart, :], x0.astype(_BF16), nt,
                                     preferred_element_type=_F32)
            y2 = jax.lax.dot_general(fe[quart:half, :], x2.astype(_BF16), nt,
                                     preferred_element_type=_F32)
            yo = jax.lax.dot_general(fo[...], xo.astype(_BF16), nt, preferred_element_type=_F32)
            top = y0[eight:eight + 8]
            re = jnp.concatenate([y0[0:eight], y2[0:eight], jnp.where(first, top, 0.0)], axis=0)
            im = jnp.concatenate([jnp.where(first, 0.0, top), y0[eight + 8:quart], y2[eight:quart],
                                  jnp.zeros((8, N2), _F32)], axis=0)
            ze[n1] = fwd_s(n1, jnp.concatenate([re, im], axis=1))
            zo[n1, :, 0:N2] = yo[0:quart]
            zo[n1, :, N2:2 * N2] = yo[quart:half]
        return 0
    jax.lax.fori_loop(0, _R // 2, fwd_d, 0)

    for c in f_copies:
        c.wait()
    filt(ze, slice(quart, quart + 8),
         [[jnp.where(first, ref[0:8, l1 * N2:(l1 + 1) * N2].astype(_F32) * 0.5, 0.0)
           for ref in (wrn_ref, win_ref)] for l1 in range(_R)])
    assert eight // 8 == _R

    def mid_e(i, _):
        for n1 in (2 * i, 2 * i + 1):
            zo[n1] = fwd_s(n1, zo[n1])
            for c in range(2):
                filt_rows(ze, 0, c, n1)
        return 0
    jax.lax.fori_loop(0, _R // 2, mid_e, 0)

    def mid_o(i, _):
        for n1 in (2 * i, 2 * i + 1):
            ze[n1, 0:quart, :] = inv_s(gmat(n1), ze[n1, 0:quart, :])
            for c in range(2):
                filt_rows(zo, 1, c, n1)
        return 0
    jax.lax.fori_loop(0, _R // 2, mid_o, 0)

    def inv_d(a, _):
        arrived(2 * a)
        arrived(2 * a + 1)
        ys = []
        for b in range(2):
            n1 = 2 * a + b
            gm = gmat(n1)
            un = inv_s(gm[0:N2], jnp.concatenate(
                [ze[n1, quart:quart + 8, :], jnp.zeros((N2 - 8, 2 * N2), _F32)], axis=0))
            uo = inv_s(gm, zo[n1])
            u0 = jnp.concatenate([ze[n1, 0:N2, 0:eight],
                                  jnp.where(lane0, un, ze[n1, N2:2 * N2, 0:eight])], axis=1)
            u2 = jnp.concatenate([ze[n1, 0:N2, eight:quart], ze[n1, N2:2 * N2, eight:quart]], axis=1)
            p2 = jnp.dot(u2, fe[quart:half, :], preferred_element_type=_F32)
            p0 = jnp.dot(u0, fe[0:quart, :], preferred_element_type=_F32)
            p = jnp.concatenate([p0 + p2, p0 - p2], axis=1)
            q = jnp.dot(jnp.concatenate([uo[0:N2], uo[N2:2 * N2]], axis=1), fo[...],
                        preferred_element_type=_F32)
            ys.append(jnp.concatenate([p + q, p - q], axis=1))
        relayout(2 * a, 2)
        bx[a] = pltpu.bitcast(pltpu.pack_elementwise(ys, packed_dtype=_BF16), _U32)
        return 0
    jax.lax.fori_loop(0, _R // 2, inv_d, 0)

    in_copies[4].wait()
    hbuf[0:M, :] = mem0_ref[...].astype(_F32)
    hbuf[M:L, :] = ax[0].astype(_F32)
    nseg = S // seg
    scale = float(np.asarray(128.0 ** -0.5, np.float32).astype(_BF16).astype(np.float32))
    neg = float(np.asarray(-1e9, np.float32).astype(_BF16).astype(np.float32))

    row = jax.lax.broadcasted_iota(jnp.int32, (L, 128), 0)
    col = jax.lax.broadcasted_iota(jnp.int32, (L, 128), 1)
    allowed = (col < L) & ((row < M) | (row >= col))
    fill = jnp.where(col < L, jnp.float32(neg), jnp.float32(-np.inf))

    def unit(m, h):
        return (h // G) * 3 + (1, 0, 2)[m]

    def weights(m, heads):
        return pltpu.bitcast(jnp.concatenate([wqkv[m, h] for h in heads], axis=1), _BF16)

    def proj(m, heads, s):
        if s is None or unit(m, heads[0]) >= _NPRE:
            y = jnp.dot(hbuf[...], weights(m, heads), preferred_element_type=_F32)
            return [y[:, i * 128:(i + 1) * 128] for i in range(len(heads))]
        y = jnp.dot(hbuf[0:L - 8, :], weights(m, heads), preferred_element_type=_F32)
        rows = pl.ds(pl.multiple_of(s * 8, 8), 8)
        return [jnp.concatenate([y[:, i * 128:(i + 1) * 128], pre[unit(m, h), h % G, rows, :]], axis=0)
                for i, h in enumerate(heads)]

    def pad_keys(t):
        return jnp.concatenate([t, jnp.zeros((128 - L, 128), _F32)], axis=0).astype(_BF16)

    def probs(q, k):
        s = jax.lax.dot_general(q, pad_keys(k), (((1,), (1,)), ((), ())),
                                preferred_element_type=_F32)
        s = jnp.where(allowed, s * scale, fill)
        e = jnp.exp(s - jnp.max(s, axis=1, keepdims=True))
        den = jnp.sum(e, axis=1, keepdims=True)
        r = pl.reciprocal(den, approx=True)
        return e * (r * (2.0 - den * r))

    def out_part(gi, n0, n1):
        c0, c1 = gi * G * 128, (gi + 1) * G * 128
        w = pltpu.bitcast(wo[c0 // 2:c1 // 2, n0:n1], _BF16)
        y = jnp.dot(obuf[:, c0:c1], w, preferred_element_type=_F32)
        if gi == 0:
            acc[:, n0:n1] = y
        else:
            acc[:, n0:n1] += y

    def values(heads, ps, vs):
        for h, p, v in zip(heads, ps, vs):
            obuf[:, h * 128:(h + 1) * 128] = jnp.dot(p, pad_keys(v), preferred_element_type=_F32)

    def group(s, gi, late):
        heads = list(range(gi * G, (gi + 1) * G))
        ks = proj(1, heads, s)
        if late is not None:
            values(*late)
        qs = proj(0, heads, s)
        vs = proj(2, heads[:2], s)
        ps = [probs(q, k) for q, k in zip(qs, ks)]
        vs += proj(2, heads[2:], s)
        if gi == 0:
            return heads, ps, vs
        out_part(gi - 1, 0, 768)
        values(heads, ps, vs)
        out_part(gi - 1, 768, D)

    def ao_copy(s):
        nb = seg // _R
        return pltpu.make_async_copy(aout.at[pl.ds(s * nb, nb)],
                                     out_hbm.at[pl.ds(s * nb, nb), :, 0:D], sem_ao)

    def emit(s):
        nb = seg // _R
        for i in range(nb):
            aout[s * nb + i] = acc[M + i * _R:M + (i + 1) * _R, :].astype(_BF16)
        ao_copy(s).start()


    in_copies[6].wait()
    for u in range(_NPRE):
        m, gi = (1, 0, 2)[u % 3], u // 3

        def ahead(i, _, m=m, gi=gi, u=u):
            arrived(_R + 4 * u + 2 * i)
            arrived(_R + 4 * u + 2 * i + 1)
            xt = xtail[...].astype(_F32).reshape(nseg * 8, D)
            heads = [gi * G + 2 * i, gi * G + 2 * i + 1]
            y = jnp.dot(xt, weights(m, heads), preferred_element_type=_F32)
            pre[u, 2 * i] = y[:, 0:128]
            pre[u, 2 * i + 1] = y[:, 128:256]
            relayout(_R + 4 * u + 2 * i, 1)
            relayout(_R + 4 * u + 2 * i + 1, 1)
            return 0
        jax.lax.fori_loop(0, G // 2, ahead, 0)

    done, last = _R + 4 * _NPRE, 6 * (ngroup - 1)
    assert 6 * -(-_NPRE // 3) <= _R and done <= last
    for p in range(done, last):
        arrived(p)
    for gi in range(ngroup - 1):
        wo_copy(gi).wait()
    late = None
    for gi in range(ngroup):
        if gi == ngroup - 2:
            for p in range(last, last + 6):
                arrived(p)
            wo_copy(ngroup - 1).wait()
        late = group(None, gi, late)
        for p in range(done, last) if gi == 0 else range(last, last + 6) if gi == ngroup - 2 else ():
            relayout(p, 1)
    out_part(ngroup - 1, 0, D)
    in_copies[5].start()
    for a in range(_R // 2):
        bo_copy(a).start()
    hbuf[M:L, :] = ax[1].astype(_F32)
    hbuf[0:M, :] = acc[0:M, :]

    def step(s, _):
        late = None
        for gi in range(ngroup):
            late = group(s, gi, late)
            if gi == 0:
                emit(s - 1)
        hbuf[M:L, :] = ax[jnp.minimum(s + 1, nseg - 1)].astype(_F32)
        out_part(ngroup - 1, 0, D)
        hbuf[0:M, :] = acc[0:M, :]
        return 0
    step(1, 0)
    in_copies[5].wait()
    jax.lax.fori_loop(2, nseg, step, 0, unroll=2)
    emit(nseg - 1)

    pltpu.make_async_copy(aout, out_hbm.at[:, :, 0:D], sem_ao).wait()
    for a in range(_R // 2):
        bo_copy(a).wait()


@functools.partial(jax.jit, static_argnames=("A_seg_len",))
def pallas_concat_heads__memory_aug_recurrent_mem_tr__spectral_gfnet__prompt_kernel(
    A_x, A_mem0, A_Wq, A_Wk, A_Wv, A_Wo, A_seg_len, B_x, B_w_r, B_w_i,
):
    _, S, D = A_x.shape
    H, Dh = A_Wq.shape[1], A_Wq.shape[2]
    M = A_mem0.shape[1]
    seg = int(A_seg_len)
    assert (S, D, H, Dh, M, seg) == (2048, 1024, 32, 128, 8, 32) and B_x.shape == (1, S, D)
    L = M + seg
    half = D // 2
    N2 = S // _R
    fo, fe, g = _dft_constants(S, D)
    wr_t, wi_t = B_w_r.T, B_w_i.T
    nyq = pl.BlockSpec((16, S), lambda i: (half // 16, 0))

    hbm = pl.BlockSpec(memory_space=pl.ANY)
    vm = pltpu.VMEM
    out = pl.pallas_call(
        functools.partial(_kernel, S=S, D=D, H=H, M=M, seg=seg),
        out_shape=jax.ShapeDtypeStruct((N2, _R, 2 * D), _BF16),
        grid=(1,),
        in_specs=[hbm, pl.BlockSpec(memory_space=pltpu.VMEM)] + [hbm] * 7 + [nyq, nyq, hbm, hbm, hbm],
        out_specs=hbm,
        scratch_shapes=[
            vm((S // seg, seg, D), _BF16),
            vm((S // seg, 8, D), _BF16),
            vm((max(_NPRE, 1), 4, S // seg * 8, Dh), _F32),
            vm((3 * H // 2, D, Dh), _U32),
            vm((3, H, D // 2, Dh), _U32),
            vm((H * Dh // 2, D), _U32),
            vm((L, D), _F32),
            vm((L, H * Dh), _F32),
            vm((L, D), _F32),
            vm((N2, _R, D), _BF16),
            vm((_R // 2, N2, D), _U32),
            vm((_R, half // 2, N2), _U32),
            vm((_R, half // 2, N2), _U32),
            vm((half, half), _BF16),
            vm((half, half // 2), _BF16),
            vm((_R, 2, 2 * N2, N2), _BF16),
            vm((_R, half // 2 + 8, 2 * N2), _F32),
            vm((_R, half // 2, 2 * N2), _F32),
            pltpu.SemaphoreType.DMA((7,)),
            pltpu.SemaphoreType.DMA((_R // 2,)),
            pltpu.SemaphoreType.DMA((_R // 2,)),
            pltpu.SemaphoreType.DMA((3 * H // 2,)),
            pltpu.SemaphoreType.DMA((H // 4,)),
            pltpu.SemaphoreType.DMA,
            pltpu.SemaphoreType.DMA,
        ],
        compiler_params=pltpu.CompilerParams(vmem_limit_bytes=120 * 1024 * 1024),
    )(A_x.reshape(S // seg, seg, D), A_mem0.reshape(M, D), A_Wq, A_Wk, A_Wv, A_Wo.reshape(H * Dh, D),
      B_x.reshape(N2, _R, D), wr_t, wi_t, wr_t, wi_t, fo, fe, g)
    return out.reshape(1, S, 2 * D)
```

```python
import functools

import jax
import jax.numpy as jnp
import numpy as np
import jax.experimental.pallas as pl
import jax.experimental.pallas.tpu as pltpu

_F32 = jnp.float32
_BF16 = jnp.bfloat16
_U32 = jnp.uint32

_R = 16
_NPRE = 6
_SQ = float(np.sqrt(0.5))


def _dft_constants(S, D):
    half, quart = D // 2, D // 4
    m = np.arange(D // 8, dtype=np.int64)

    def block(k, n):
        ang = 2.0 * np.pi * ((k[:, None] * np.arange(n, dtype=np.int64)[None, :]) % D) / D
        return np.concatenate([np.cos(ang), -np.sin(ang)], axis=0)

    fo = block(np.concatenate([4 * m + 1, 4 * m + 3]), half)
    f2 = block(4 * m + 2, quart)
    f0 = block(4 * m, quart)
    f0[m.size] = np.where(np.arange(quart) % 2 == 0, 1.0, -1.0)
    fe = np.concatenate([f0, f2], axis=0)
    n2 = np.arange(S // _R, dtype=np.int64)
    g = np.zeros((_R, 2 * (S // _R), 2 * (S // _R)))
    for n1 in range(_R):
        a = 2.0 * np.pi * (((n1 + _R * n2)[:, None] * n2[None, :]) % S) / S
        gr, gi = np.cos(a), -np.sin(a)
        g[n1] = np.block([[gr, gi], [-gi, gr]])
    g = g * np.sqrt(2.0 / (S * D))
    cast = lambda a: np.asarray(a, np.float32).astype(_BF16)
    g = g.reshape(_R, 2 * n2.size, 2, n2.size).transpose(0, 2, 1, 3)
    return cast(fo), cast(fe), cast(g)


def _cmul_const(z, j, n, sgn):
    re, im = z
    j %= n
    if j == 0:
        return re, im
    if 2 * j == n:
        return -re, -im
    if 4 * j == n:
        return (-im, re) if sgn > 0 else (im, -re)
    if 4 * j == 3 * n:
        return (im, -re) if sgn > 0 else (-im, re)
    c = float(np.cos(2 * np.pi * j / n))
    s = float(sgn * np.sin(2 * np.pi * j / n))
    if 8 * j % n == 0:
        a = re + im if c * s < 0 else re - im
        b = im - re if c * s < 0 else im + re
        return a * c, b * c
    return re * c - im * s, re * s + im * c


def _fft(zs, sgn):
    n = len(zs)
    if n == 1:
        return zs
    ev = _fft(zs[0::2], sgn)
    od = _fft(zs[1::2], sgn)
    out = [None] * n
    for j in range(n // 2):
        if 4 * j == n:
            (er, ei), (orr, oi) = ev[j], od[j]
            if sgn > 0:
                out[j], out[j + n // 2] = (er - oi, ei + orr), (er + oi, ei - orr)
            else:
                out[j], out[j + n // 2] = (er + oi, ei - orr), (er - oi, ei + orr)
            continue
        tr, ti = _cmul_const(od[j], j, n, sgn)
        out[j] = (ev[j][0] + tr, ev[j][1] + ti)
        out[j + n // 2] = (ev[j][0] - tr, ev[j][1] - ti)
    return out


def _halves(u):
    return (pltpu.bitcast(u << 16, _F32), pltpu.bitcast(u & jnp.uint32(0xFFFF0000), _F32))


def _kernel(ax_hbm, mem0_hbm, wq_hbm, wk_hbm, wv_hbm, wo_hbm, bx_hbm, wr_hbm, wi_hbm,
            fo_hbm, fe_hbm, g_hbm, out_hbm,
            ax, xtail, pre, stage, wqkv, wo, hbuf, obuf, acc, aout,
            mem0_ref, wrn_ref, win_ref, bx, wr, wi, fo, fe, g, ze, zo,
            sem_in, sem_x, sem_g, sem_w, sem_wo, sem_ao, sem_bo, *, S, D, H, M, seg):
    half, quart, eight = D // 2, D // 4, D // 8
    N2 = S // _R
    L = M + seg
    w_hbms = (wq_hbm, wk_hbm, wv_hbm)
    nt = (((1,), (1,)), ((), ()))

    in_copies = [
        pltpu.make_async_copy(fo_hbm, fo, sem_in.at[0]),
        pltpu.make_async_copy(fe_hbm, fe, sem_in.at[1]),
        pltpu.make_async_copy(wr_hbm.at[half:half + 1], wrn_ref, sem_in.at[2]),
        pltpu.make_async_copy(wi_hbm.at[half:half + 1], win_ref, sem_in.at[2]),
        pltpu.make_async_copy(ax_hbm.at[0:8], ax.at[0:8], sem_in.at[4]),
        pltpu.make_async_copy(ax_hbm.at[8:S // seg], ax.at[8:S // seg], sem_in.at[5]),
        pltpu.make_async_copy(ax_hbm.at[:, seg - 8:seg], xtail, sem_in.at[6]),
        pltpu.make_async_copy(mem0_hbm, mem0_ref, sem_in.at[3]),
    ]
    G = 4
    ngroup = H // G

    def wo_copy(gi):
        rows = pl.ds(pl.multiple_of(gi * G * 64, G * 64), G * 64)
        return pltpu.make_async_copy(wo_hbm.bitcast(_U32).at[rows], wo.at[rows], sem_wo.at[gi])

    def bo_copy(a):
        return pltpu.make_async_copy(bx.at[a], out_hbm.bitcast(_U32).at[:, a, D:2 * D], sem_bo)

    def x_copy(a):
        return pltpu.make_async_copy(bx_hbm.bitcast(_U32).at[:, a, :], bx.at[a], sem_x.at[a])

    def w_copy(m, j):
        return pltpu.make_async_copy(w_hbms[m].bitcast(_U32).at[:, j, :],
                                     stage.at[3 * j + m], sem_w.at[3 * j + m])

    def arrived(p):
        pltpu.make_async_copy(stage.at[p], stage.at[p], sem_w.at[p]).wait()

    def relayout(p0, n):
        words = [[stage[p0 + i, pl.ds(r, half, stride=2), :] for r in range(2)] for i in range(n)]
        for i, (ev, od) in enumerate(words):
            j, m = (p0 + i) // 3, (p0 + i) % 3
            wqkv[m, 2 * j] = (ev & jnp.uint32(0xFFFF)) | (od << 16)
            wqkv[m, 2 * j + 1] = (ev >> 16) | (od & jnp.uint32(0xFFFF0000))

    def g_copy(a):
        return pltpu.make_async_copy(g_hbm.at[pl.ds(2 * a, 2)], g.at[pl.ds(2 * a, 2)], sem_g.at[a])

    x_copy(0).start()
    in_copies[0].start()
    in_copies[1].start()
    g_copy(0).start()
    for a in range(1, _R // 2):
        x_copy(a).start()
        g_copy(a).start()
    in_copies[0].wait()
    in_copies[1].wait()
    f_copies = [
        pltpu.make_async_copy(src.at[0:half].bitcast(_U32).at[:, l1 * N2:(l1 + 1) * N2],
                              dst.at[l1], sem_in.at[2])
        for src, dst in ((wr_hbm, wr), (wi_hbm, wi)) for l1 in range(_R)] + in_copies[2:4]
    for c in f_copies + [in_copies[4], in_copies[6], in_copies[7]]:
        c.start()

    first = jax.lax.broadcasted_iota(jnp.int32, (8, N2), 0) == 0
    lane0 = jax.lax.broadcasted_iota(jnp.int32, (N2, N2), 1) == 0

    def gmat(n1):
        return jnp.concatenate([g[n1, 0], g[n1, 1]], axis=1)

    def fwd_s(n1, zt):
        return jnp.dot(zt, gmat(n1), preferred_element_type=_F32)

    def inv_s(gm, yt):
        return jax.lax.dot_general(gm, yt, nt, preferred_element_type=_F32)

    def filt(zr, rows, ws):
        xs = _fft([(zr[n, rows, 0:N2], zr[n, rows, N2:2 * N2]) for n in range(_R)], -1)
        ys = [(xr * fr - xi * fi, xr * fi + xi * fr) for (xr, xi), (fr, fi) in zip(xs, ws)]
        for n, (yr, yi) in enumerate(_fft(ys, +1)):
            zr[n, rows, 0:N2] = yr
            zr[n, rows, N2:2 * N2] = yi

    def filt_rows(zr, par, c, j):
        rows = pl.ds(pl.multiple_of(c * eight + j * 8, 8), 8)
        ws = [[_halves(ref[l1, pl.ds(16 * j + c, 8, stride=2), :])[par] for ref in (wr, wi)]
              for l1 in range(_R)]
        if par == 0 and c == 0:
            dc = jnp.where(first & (j == 0), 0.5, 1.0)
            ws = [[w * dc for w in f] for f in ws]
        filt(zr, rows, ws)

    assert ngroup == _R // 2

    def fwd_d(a, _):
        for j in range(G // 2):
            for m in range(3):
                w_copy(m, a * (G // 2) + j).start()
        wo_copy(a).start()
        x_copy(a).wait()
        g_copy(a).wait()
        for b, x in enumerate(_halves(bx[a])):
            n1 = 2 * a + b
            xe, xo = x[:, 0:half] + x[:, half:D], x[:, 0:half] - x[:, half:D]
            x0, x2 = xe[:, 0:quart] + xe[:, quart:half], xe[:, 0:quart] - xe[:, quart:half]
            y0 = jax.lax.dot_general(fe[0:quart, :], x0.astype(_BF16), nt,
                                     preferred_element_type=_F32)
            y2 = jax.lax.dot_general(fe[quart:half, :], x2.astype(_BF16), nt,
                                     preferred_element_type=_F32)
            yo = jax.lax.dot_general(fo[...], xo.astype(_BF16), nt, preferred_element_type=_F32)
            top = y0[eight:eight + 8]
            re = jnp.concatenate([y0[0:eight], y2[0:eight], jnp.where(first, top, 0.0)], axis=0)
            im = jnp.concatenate([jnp.where(first, 0.0, top), y0[eight + 8:quart], y2[eight:quart],
                                  jnp.zeros((8, N2), _F32)], axis=0)
            ze[n1] = fwd_s(n1, jnp.concatenate([re, im], axis=1))
            zo[n1, :, 0:N2] = yo[0:quart]
            zo[n1, :, N2:2 * N2] = yo[quart:half]
        return 0
    jax.lax.fori_loop(0, _R // 2, fwd_d, 0)

    for c in f_copies:
        c.wait()
    filt(ze, slice(quart, quart + 8),
         [[jnp.where(first, ref[:, l1 * N2:(l1 + 1) * N2].astype(_F32) * 0.5, 0.0)
           for ref in (wrn_ref, win_ref)] for l1 in range(_R)])
    assert eight // 8 == _R

    def mid_e(i, _):
        for n1 in (2 * i, 2 * i + 1):
            zo[n1] = fwd_s(n1, zo[n1])
            for c in range(2):
                filt_rows(ze, 0, c, n1)
        return 0
    jax.lax.fori_loop(0, _R // 2, mid_e, 0)

    def mid_o(i, _):
        for n1 in (2 * i, 2 * i + 1):
            ze[n1, 0:quart, :] = inv_s(gmat(n1), ze[n1, 0:quart, :])
            for c in range(2):
                filt_rows(zo, 1, c, n1)
        return 0
    jax.lax.fori_loop(0, _R // 2, mid_o, 0)

    def inv_d(a, _):
        arrived(2 * a)
        arrived(2 * a + 1)
        ys = []
        for b in range(2):
            n1 = 2 * a + b
            gm = gmat(n1)
            un = inv_s(gm[0:N2], jnp.concatenate(
                [ze[n1, quart:quart + 8, :], jnp.zeros((N2 - 8, 2 * N2), _F32)], axis=0))
            uo = inv_s(gm, zo[n1])
            u0 = jnp.concatenate([ze[n1, 0:N2, 0:eight],
                                  jnp.where(lane0, un, ze[n1, N2:2 * N2, 0:eight])], axis=1)
            u2 = jnp.concatenate([ze[n1, 0:N2, eight:quart], ze[n1, N2:2 * N2, eight:quart]], axis=1)
            p2 = jnp.dot(u2, fe[quart:half, :], preferred_element_type=_F32)
            p0 = jnp.dot(u0, fe[0:quart, :], preferred_element_type=_F32)
            p = jnp.concatenate([p0 + p2, p0 - p2], axis=1)
            q = jnp.dot(jnp.concatenate([uo[0:N2], uo[N2:2 * N2]], axis=1), fo[...],
                        preferred_element_type=_F32)
            ys.append(jnp.concatenate([p + q, p - q], axis=1))
        relayout(2 * a, 2)
        lo, hi = [pltpu.bitcast(y.astype(_BF16).astype(_F32), _U32) for y in ys]
        bx[a] = (lo >> 16) | hi
        return 0
    jax.lax.fori_loop(0, _R // 2, inv_d, 0)

    in_copies[4].wait()
    in_copies[7].wait()
    hbuf[0:M, :] = mem0_ref[...].astype(_F32)
    hbuf[M:L, :] = ax[0].astype(_F32)
    nseg = S // seg
    scale = float(np.asarray(128.0 ** -0.5, np.float32).astype(_BF16).astype(np.float32))
    neg = float(np.asarray(-1e9, np.float32).astype(_BF16).astype(np.float32))

    row = jax.lax.broadcasted_iota(jnp.int32, (L, 128), 0)
    col = jax.lax.broadcasted_iota(jnp.int32, (L, 128), 1)
    allowed = (col < L) & ((row < M) | (row >= col))
    fill = jnp.where(col < L, jnp.float32(neg), jnp.float32(-np.inf))

    def unit(m, h):
        return (h // G) * 3 + (1, 0, 2)[m]

    def weights(m, heads):
        return pltpu.bitcast(jnp.concatenate([wqkv[m, h] for h in heads], axis=1), _BF16)

    def proj(m, heads, s):
        if s is None or unit(m, heads[0]) >= _NPRE:
            y = jnp.dot(hbuf[...], weights(m, heads), preferred_element_type=_F32)
            return [y[:, i * 128:(i + 1) * 128] for i in range(len(heads))]
        y = jnp.dot(hbuf[0:L - 8, :], weights(m, heads), preferred_element_type=_F32)
        rows = pl.ds(pl.multiple_of(s * 8, 8), 8)
        return [jnp.concatenate([y[:, i * 128:(i + 1) * 128], pre[unit(m, h), h % G, rows, :]], axis=0)
                for i, h in enumerate(heads)]

    def pad_keys(t):
        return jnp.concatenate([t, jnp.zeros((128 - L, 128), _F32)], axis=0).astype(_BF16)

    def probs(q, k):
        s = jax.lax.dot_general(q, pad_keys(k), (((1,), (1,)), ((), ())),
                                preferred_element_type=_F32)
        s = jnp.where(allowed, s * scale, fill)
        e = jnp.exp(s - jnp.max(s, axis=1, keepdims=True))
        den = jnp.sum(e, axis=1, keepdims=True)
        r = pl.reciprocal(den, approx=True)
        return e * (r * (2.0 - den * r))

    def out_part(gi, n0, n1):
        c0, c1 = gi * G * 128, (gi + 1) * G * 128
        w = pltpu.bitcast(wo[c0 // 2:c1 // 2, n0:n1], _BF16)
        y = jnp.dot(obuf[:, c0:c1], w, preferred_element_type=_F32)
        if gi == 0:
            acc[:, n0:n1] = y
        else:
            acc[:, n0:n1] += y

    def values(heads, ps, vs):
        for h, p, v in zip(heads, ps, vs):
            obuf[:, h * 128:(h + 1) * 128] = jnp.dot(p, pad_keys(v), preferred_element_type=_F32)

    def group(s, gi, late):
        heads = list(range(gi * G, (gi + 1) * G))
        ks = proj(1, heads, s)
        if late is not None:
            values(*late)
        qs = proj(0, heads, s)
        vs = proj(2, heads[:2], s)
        ps = [probs(q, k) for q, k in zip(qs, ks)]
        vs += proj(2, heads[2:], s)
        if gi == 0:
            return heads, ps, vs
        out_part(gi - 1, 0, 768)
        values(heads, ps, vs)
        out_part(gi - 1, 768, D)

    def ao_copy(s):
        nb = seg // _R
        return pltpu.make_async_copy(aout.at[pl.ds(s * nb, nb)],
                                     out_hbm.at[pl.ds(s * nb, nb), :, 0:D], sem_ao)

    def emit(s):
        nb = seg // _R
        for i in range(nb):
            aout[s * nb + i] = acc[M + i * _R:M + (i + 1) * _R, :].astype(_BF16)
        ao_copy(s).start()

    in_copies[6].wait()

    def ahead(it, _):
        u, i = it // 2, it % 2
        m = jnp.where(u % 3 == 2, 2, 1 - u % 3)
        h0 = (u // 3) * G + 2 * i
        arrived(_R + 2 * it)
        arrived(_R + 2 * it + 1)
        y = jnp.dot(xtail[...].astype(_F32).reshape(nseg * 8, D), weights(m, [h0, h0 + 1]),
                    preferred_element_type=_F32)
        pre[u, 2 * i] = y[:, 0:128]
        pre[u, 2 * i + 1] = y[:, 128:256]
        relayout(_R + 2 * it, 2)
        return 0
    jax.lax.fori_loop(0, 2 * _NPRE, ahead, 0)

    done, last = _R + 4 * _NPRE, 6 * (ngroup - 1)
    assert 6 * -(-_NPRE // 3) <= _R and done <= last
    for p in range(done, last):
        arrived(p)
    for gi in range(ngroup - 1):
        wo_copy(gi).wait()
    late = None
    for gi in range(ngroup):
        if gi == ngroup - 2:
            for p in range(last, last + 6):
                arrived(p)
            wo_copy(ngroup - 1).wait()
        late = group(None, gi, late)
        for p in range(done, last) if gi == 0 else range(last, last + 6) if gi == ngroup - 2 else ():
            relayout(p, 1)
    out_part(ngroup - 1, 0, D)
    in_copies[5].start()
    for a in range(_R // 2):
        bo_copy(a).start()
    hbuf[M:L, :] = ax[1].astype(_F32)
    hbuf[0:M, :] = acc[0:M, :]

    def step(s, _):
        late = None
        for gi in range(ngroup):
            late = group(s, gi, late)
            if gi == 0:
                emit(s - 1)
        hbuf[M:L, :] = ax[jnp.minimum(s + 1, nseg - 1)].astype(_F32)
        out_part(ngroup - 1, 0, D)
        hbuf[0:M, :] = acc[0:M, :]
        return 0
    step(1, 0)
    in_copies[5].wait()
    jax.lax.fori_loop(2, nseg, step, 0, unroll=2)
    emit(nseg - 1)

    pltpu.make_async_copy(aout, out_hbm.at[:, :, 0:D], sem_ao).wait()
    for a in range(_R // 2):
        bo_copy(a).wait()


@functools.partial(jax.jit, static_argnames=("A_seg_len",))
def pallas_concat_heads__memory_aug_recurrent_mem_tr__spectral_gfnet__prompt_kernel(
    A_x, A_mem0, A_Wq, A_Wk, A_Wv, A_Wo, A_seg_len, B_x, B_w_r, B_w_i,
):
    _, S, D = A_x.shape
    H, Dh = A_Wq.shape[1], A_Wq.shape[2]
    M = A_mem0.shape[1]
    seg = int(A_seg_len)
    assert (S, D, H, Dh, M, seg) == (2048, 1024, 32, 128, 8, 32) and B_x.shape == (1, S, D)
    L = M + seg
    half = D // 2
    N2 = S // _R
    fo, fe, g = _dft_constants(S, D)
    wr_t, wi_t = B_w_r.T, B_w_i.T

    hbm = pl.BlockSpec(memory_space=pl.ANY)
    vm = pltpu.VMEM
    out = pl.pallas_call(
        functools.partial(_kernel, S=S, D=D, H=H, M=M, seg=seg),
        out_shape=jax.ShapeDtypeStruct((N2, _R, 2 * D), _BF16),
        in_specs=[hbm] * 12,
        out_specs=hbm,
        scratch_shapes=[
            vm((S // seg, seg, D), _BF16),
            vm((S // seg, 8, D), _BF16),
            vm((max(_NPRE, 1), 4, S // seg * 8, Dh), _F32),
            vm((3 * H // 2, D, Dh), _U32),
            vm((3, H, D // 2, Dh), _U32),
            vm((H * Dh // 2, D), _U32),
            vm((L, D), _F32),
            vm((L, H * Dh), _F32),
            vm((L, D), _F32),
            vm((N2, _R, D), _BF16),
            vm((M, D), _BF16),
            vm((1, S), _BF16),
            vm((1, S), _BF16),
            vm((_R // 2, N2, D), _U32),
            vm((_R, half // 2, N2), _U32),
            vm((_R, half // 2, N2), _U32),
            vm((half, half), _BF16),
            vm((half, half // 2), _BF16),
            vm((_R, 2, 2 * N2, N2), _BF16),
            vm((_R, half // 2 + 8, 2 * N2), _F32),
            vm((_R, half // 2, 2 * N2), _F32),
            pltpu.SemaphoreType.DMA((7,)),
            pltpu.SemaphoreType.DMA((_R // 2,)),
            pltpu.SemaphoreType.DMA((_R // 2,)),
            pltpu.SemaphoreType.DMA((3 * H // 2,)),
            pltpu.SemaphoreType.DMA((H // 4,)),
            pltpu.SemaphoreType.DMA,
            pltpu.SemaphoreType.DMA,
        ],
        compiler_params=pltpu.CompilerParams(vmem_limit_bytes=120 * 1024 * 1024),
    )(A_x.reshape(S // seg, seg, D), A_mem0.reshape(M, D), A_Wq, A_Wk, A_Wv, A_Wo.reshape(H * Dh, D),
      B_x.reshape(N2, _R, D), wr_t, wi_t, fo, fe, g)
    return out.reshape(1, S, 2 * D)
```

```python
import functools

import jax
import jax.numpy as jnp
import numpy as np
import jax.experimental.pallas as pl
import jax.experimental.pallas.tpu as pltpu

_F32 = jnp.float32
_BF16 = jnp.bfloat16
_U32 = jnp.uint32

_R = 16
_NPRE = 6
_SQ = float(np.sqrt(0.5))


def _dft_constants(S, D):
    half, quart = D // 2, D // 4
    m = np.arange(D // 8, dtype=np.int64)

    def block(k, n):
        ang = 2.0 * np.pi * ((k[:, None] * np.arange(n, dtype=np.int64)[None, :]) % D) / D
        return np.concatenate([np.cos(ang), -np.sin(ang)], axis=0)

    fo = block(np.concatenate([4 * m + 1, 4 * m + 3]), half)
    f2 = block(4 * m + 2, quart)
    f0 = block(4 * m, quart)
    f0[m.size] = np.where(np.arange(quart) % 2 == 0, 1.0, -1.0)
    fe = np.concatenate([f0, f2], axis=0)
    n2 = np.arange(S // _R, dtype=np.int64)
    g = np.zeros((_R, 2 * (S // _R), 2 * (S // _R)))
    for n1 in range(_R):
        a = 2.0 * np.pi * (((n1 + _R * n2)[:, None] * n2[None, :]) % S) / S
        gr, gi = np.cos(a), -np.sin(a)
        g[n1] = np.block([[gr, gi], [-gi, gr]])
    g = g * np.sqrt(2.0 / (S * D))
    cast = lambda a: np.asarray(a, np.float32).astype(_BF16)
    g = g.reshape(_R, 2 * n2.size, 2, n2.size).transpose(0, 2, 1, 3)
    return cast(fo), cast(fe), cast(g)


def _cmul_const(z, j, n, sgn):
    re, im = z
    j %= n
    if j == 0:
        return re, im
    if 2 * j == n:
        return -re, -im
    if 4 * j == n:
        return (-im, re) if sgn > 0 else (im, -re)
    if 4 * j == 3 * n:
        return (im, -re) if sgn > 0 else (-im, re)
    c = float(np.cos(2 * np.pi * j / n))
    s = float(sgn * np.sin(2 * np.pi * j / n))
    if 8 * j % n == 0:
        a = re + im if c * s < 0 else re - im
        b = im - re if c * s < 0 else im + re
        return a * c, b * c
    return re * c - im * s, re * s + im * c


def _fft(zs, sgn):
    n = len(zs)
    if n == 1:
        return zs
    ev = _fft(zs[0::2], sgn)
    od = _fft(zs[1::2], sgn)
    out = [None] * n
    for j in range(n // 2):
        if 4 * j == n:
            (er, ei), (orr, oi) = ev[j], od[j]
            if sgn > 0:
                out[j], out[j + n // 2] = (er - oi, ei + orr), (er + oi, ei - orr)
            else:
                out[j], out[j + n // 2] = (er + oi, ei - orr), (er - oi, ei + orr)
            continue
        tr, ti = _cmul_const(od[j], j, n, sgn)
        out[j] = (ev[j][0] + tr, ev[j][1] + ti)
        out[j + n // 2] = (ev[j][0] - tr, ev[j][1] - ti)
    return out


def _halves(u):
    return (pltpu.bitcast(u << 16, _F32), pltpu.bitcast(u & jnp.uint32(0xFFFF0000), _F32))


def _kernel(ax_hbm, mem0_hbm, wq_hbm, wk_hbm, wv_hbm, wo_hbm, bx_hbm, wr_hbm, wi_hbm,
            fo_hbm, fe_hbm, g_hbm, out_hbm,
            ax, xtail, pre, stage, wqkv, wo, hbuf, obuf, acc, aout,
            mem0_ref, wrn_ref, win_ref, bx, wr, wi, fo, fe, g, ze, zo,
            sem_in, sem_x, sem_g, sem_w, sem_wo, sem_ao, sem_bo, *, S, D, H, M, seg):
    half, quart, eight = D // 2, D // 4, D // 8
    N2 = S // _R
    L = M + seg
    w_hbms = (wq_hbm, wk_hbm, wv_hbm)
    nt = (((1,), (1,)), ((), ()))

    in_copies = [
        pltpu.make_async_copy(fo_hbm, fo, sem_in.at[0]),
        pltpu.make_async_copy(fe_hbm, fe, sem_in.at[1]),
        pltpu.make_async_copy(wr_hbm.at[half:half + 1], wrn_ref, sem_in.at[2]),
        pltpu.make_async_copy(wi_hbm.at[half:half + 1], win_ref, sem_in.at[2]),
        pltpu.make_async_copy(ax_hbm.at[0:8], ax.at[0:8], sem_in.at[4]),
        pltpu.make_async_copy(ax_hbm.at[8:S // seg], ax.at[8:S // seg], sem_in.at[5]),
        pltpu.make_async_copy(ax_hbm.at[:, seg - 8:seg], xtail, sem_in.at[6]),
        pltpu.make_async_copy(mem0_hbm, mem0_ref, sem_in.at[3]),
    ]
    G = 4
    ngroup = H // G

    def wo_copy(gi):
        rows = pl.ds(pl.multiple_of(gi * G * 64, G * 64), G * 64)
        return pltpu.make_async_copy(wo_hbm.bitcast(_U32).at[rows], wo.at[rows], sem_wo.at[gi])

    def bo_copy(a):
        return pltpu.make_async_copy(bx.at[a], out_hbm.bitcast(_U32).at[:, a, D:2 * D], sem_bo)

    def x_copy(a):
        return pltpu.make_async_copy(bx_hbm.bitcast(_U32).at[:, a, :], bx.at[a], sem_x.at[a])

    def w_copy(m, j):
        return pltpu.make_async_copy(w_hbms[m].bitcast(_U32).at[:, j, :],
                                     stage.at[3 * j + m], sem_w.at[3 * j + m])

    def arrived(p):
        pltpu.make_async_copy(stage.at[p], stage.at[p], sem_w.at[p]).wait()

    def relayout(p0, n):
        words = [[stage[p0 + i, pl.ds(r, half, stride=2), :] for r in range(2)] for i in range(n)]
        for i, (ev, od) in enumerate(words):
            j, m = (p0 + i) // 3, (p0 + i) % 3
            wqkv[m, 2 * j] = (ev & jnp.uint32(0xFFFF)) | (od << 16)
            wqkv[m, 2 * j + 1] = (ev >> 16) | (od & jnp.uint32(0xFFFF0000))

    def g_copy(a):
        return pltpu.make_async_copy(g_hbm.at[pl.ds(2 * a, 2)], g.at[pl.ds(2 * a, 2)], sem_g.at[a])

    x_copy(0).start()
    in_copies[0].start()
    in_copies[1].start()
    g_copy(0).start()
    for a in range(1, _R // 2):
        x_copy(a).start()
        g_copy(a).start()
    in_copies[0].wait()
    in_copies[1].wait()
    f_copies = [
        pltpu.make_async_copy(src.at[0:half].bitcast(_U32).at[:, l1 * N2:(l1 + 1) * N2],
                              dst.at[l1], sem_in.at[2])
        for src, dst in ((wr_hbm, wr), (wi_hbm, wi)) for l1 in range(_R)] + in_copies[2:4]
    for c in f_copies + [in_copies[4], in_copies[6], in_copies[7]]:
        c.start()

    first = jax.lax.broadcasted_iota(jnp.int32, (8, N2), 0) == 0
    lane0 = jax.lax.broadcasted_iota(jnp.int32, (N2, N2), 1) == 0

    def gmat(n1):
        return jnp.concatenate([g[n1, 0], g[n1, 1]], axis=1)

    def fwd_s(n1, zt):
        return jnp.dot(zt, gmat(n1), preferred_element_type=_F32)

    def inv_s(gm, yt):
        return jax.lax.dot_general(gm, yt, nt, preferred_element_type=_F32)

    def filt(zr, rows, ws):
        xs = _fft([(zr[n, rows, 0:N2], zr[n, rows, N2:2 * N2]) for n in range(_R)], -1)
        ys = [(xr * fr - xi * fi, xr * fi + xi * fr) for (xr, xi), (fr, fi) in zip(xs, ws)]
        for n, (yr, yi) in enumerate(_fft(ys, +1)):
            zr[n, rows, 0:N2] = yr
            zr[n, rows, N2:2 * N2] = yi

    def filt_rows(zr, par, c, j):
        rows = pl.ds(pl.multiple_of(c * eight + j * 8, 8), 8)
        ws = [[_halves(ref[l1, pl.ds(16 * j + c, 8, stride=2), :])[par] for ref in (wr, wi)]
              for l1 in range(_R)]
        if par == 0 and c == 0:
            dc = jnp.where(first & (j == 0), 0.5, 1.0)
            ws = [[w * dc for w in f] for f in ws]
        filt(zr, rows, ws)

    assert ngroup == _R // 2

    def fwd_d(a, _):
        for j in range(G // 2):
            for m in range(3):
                w_copy(m, a * (G // 2) + j).start()
        wo_copy(a).start()
        x_copy(a).wait()
        g_copy(a).wait()
        for b, x in enumerate(_halves(bx[a])):
            n1 = 2 * a + b
            xe, xo = x[:, 0:half] + x[:, half:D], x[:, 0:half] - x[:, half:D]
            x0, x2 = xe[:, 0:quart] + xe[:, quart:half], xe[:, 0:quart] - xe[:, quart:half]
            y0 = jax.lax.dot_general(fe[0:quart, :], x0.astype(_BF16), nt,
                                     preferred_element_type=_F32)
            y2 = jax.lax.dot_general(fe[quart:half, :], x2.astype(_BF16), nt,
                                     preferred_element_type=_F32)
            yo = jax.lax.dot_general(fo[...], xo.astype(_BF16), nt, preferred_element_type=_F32)
            top = y0[eight:eight + 8]
            re = jnp.concatenate([y0[0:eight], y2[0:eight], jnp.where(first, top, 0.0)], axis=0)
            im = jnp.concatenate([jnp.where(first, 0.0, top), y0[eight + 8:quart], y2[eight:quart],
                                  jnp.zeros((8, N2), _F32)], axis=0)
            ze[n1] = fwd_s(n1, jnp.concatenate([re, im], axis=1))
            zo[n1, :, 0:N2] = yo[0:quart]
            zo[n1, :, N2:2 * N2] = yo[quart:half]
        return 0
    jax.lax.fori_loop(0, _R // 2, fwd_d, 0)

    for c in f_copies:
        c.wait()
    filt(ze, slice(quart, quart + 8),
         [[jnp.where(first, ref[:, l1 * N2:(l1 + 1) * N2].astype(_F32) * 0.5, 0.0)
           for ref in (wrn_ref, win_ref)] for l1 in range(_R)])
    assert eight // 8 == _R

    def mid_e(i, _):
        for n1 in (2 * i, 2 * i + 1):
            zo[n1] = fwd_s(n1, zo[n1])
            for c in range(2):
                filt_rows(ze, 0, c, n1)
        return 0
    jax.lax.fori_loop(0, _R // 2, mid_e, 0)

    def mid_o(i, _):
        for n1 in (2 * i, 2 * i + 1):
            ze[n1, 0:quart, :] = inv_s(gmat(n1), ze[n1, 0:quart, :])
            for c in range(2):
                filt_rows(zo, 1, c, n1)
        return 0
    jax.lax.fori_loop(0, _R // 2, mid_o, 0)

    def inv_d(a, _):
        arrived(2 * a)
        arrived(2 * a + 1)
        ys = []
        for b in range(2):
            n1 = 2 * a + b
            gm = gmat(n1)
            un = inv_s(gm[0:N2], jnp.concatenate(
                [ze[n1, quart:quart + 8, :], jnp.zeros((N2 - 8, 2 * N2), _F32)], axis=0))
            uo = inv_s(gm, zo[n1])
            u0 = jnp.concatenate([ze[n1, 0:N2, 0:eight],
                                  jnp.where(lane0, un, ze[n1, N2:2 * N2, 0:eight])], axis=1)
            u2 = jnp.concatenate([ze[n1, 0:N2, eight:quart], ze[n1, N2:2 * N2, eight:quart]], axis=1)
            p2 = jnp.dot(u2, fe[quart:half, :], preferred_element_type=_F32)
            p0 = jnp.dot(u0, fe[0:quart, :], preferred_element_type=_F32)
            p = jnp.concatenate([p0 + p2, p0 - p2], axis=1)
            q = jnp.dot(jnp.concatenate([uo[0:N2], uo[N2:2 * N2]], axis=1), fo[...],
                        preferred_element_type=_F32)
            ys.append(jnp.concatenate([p + q, p - q], axis=1))
        relayout(2 * a, 2)
        lo, hi = [pltpu.bitcast(y.astype(_BF16).astype(_F32), _U32) for y in ys]
        bx[a] = (lo >> 16) | hi
        return 0
    jax.lax.fori_loop(0, _R // 2, inv_d, 0)

    in_copies[4].wait()
    in_copies[7].wait()
    hbuf[0:M, :] = mem0_ref[...].astype(_F32)
    hbuf[M:L, :] = ax[0].astype(_F32)
    nseg = S // seg
    scale = float(np.asarray(128.0 ** -0.5, np.float32).astype(_BF16).astype(np.float32))
    neg = float(np.asarray(-1e9, np.float32).astype(_BF16).astype(np.float32))

    row = jax.lax.broadcasted_iota(jnp.int32, (L, 128), 0)
    col = jax.lax.broadcasted_iota(jnp.int32, (L, 128), 1)
    allowed = (col < L) & ((row < M) | (row >= col))
    fill = jnp.where(col < L, jnp.float32(neg), jnp.float32(-np.inf))

    def unit(m, h):
        return (h // G) * 3 + (1, 0, 2)[m]

    def weights(m, heads):
        return pltpu.bitcast(jnp.concatenate([wqkv[m, h] for h in heads], axis=1), _BF16)

    def proj(m, heads, s):
        if s is None or unit(m, heads[0]) >= _NPRE:
            y = jnp.dot(hbuf[...], weights(m, heads), preferred_element_type=_F32)
            return [y[:, i * 128:(i + 1) * 128] for i in range(len(heads))]
        y = jnp.dot(hbuf[0:L - 8, :], weights(m, heads), preferred_element_type=_F32)
        rows = pl.ds(pl.multiple_of(s * 8, 8), 8)
        return [jnp.concatenate([y[:, i * 128:(i + 1) * 128], pre[unit(m, h), h % G, rows, :]], axis=0)
                for i, h in enumerate(heads)]

    def pad_keys(t):
        return jnp.concatenate([t, jnp.zeros((128 - L, 128), _F32)], axis=0).astype(_BF16)

    def probs(q, k):
        s = jax.lax.dot_general(q, pad_keys(k), (((1,), (1,)), ((), ())),
                                preferred_element_type=_F32)
        s = jnp.where(allowed, s * scale, fill)
        e = jnp.exp(s - jnp.max(s, axis=1, keepdims=True))
        den = jnp.sum(e, axis=1, keepdims=True)
        r = pl.reciprocal(den, approx=True)
        return e * (r * (2.0 - den * r))

    def out_part(gi, n0, n1):
        c0, c1 = gi * G * 128, (gi + 1) * G * 128
        w = pltpu.bitcast(wo[c0 // 2:c1 // 2, n0:n1], _BF16)
        y = jnp.dot(obuf[:, c0:c1], w, preferred_element_type=_F32)
        if gi == 0:
            acc[:, n0:n1] = y
        else:
            acc[:, n0:n1] += y

    def values(heads, ps, vs):
        for h, p, v in zip(heads, ps, vs):
            obuf[:, h * 128:(h + 1) * 128] = jnp.dot(p, pad_keys(v), preferred_element_type=_F32)

    def group(s, gi, late):
        heads = list(range(gi * G, (gi + 1) * G))
        ks = proj(1, heads, s)
        if late is not None:
            values(*late)
        qs = proj(0, heads, s)
        vs = proj(2, heads[:2], s)
        ps = [probs(q, k) for q, k in zip(qs, ks)]
        vs += proj(2, heads[2:], s)
        if gi == 0:
            return heads, ps, vs
        out_part(gi - 1, 0, 768)
        values(heads, ps, vs)
        out_part(gi - 1, 768, D)

    def ao_copy(s):
        nb = seg // _R
        return pltpu.make_async_copy(aout.at[pl.ds(s * nb, nb)],
                                     out_hbm.at[pl.ds(s * nb, nb), :, 0:D], sem_ao)

    def emit(s):
        nb = seg // _R
        for i in range(nb):
            aout[s * nb + i] = acc[M + i * _R:M + (i + 1) * _R, :].astype(_BF16)
        ao_copy(s).start()

    in_copies[6].wait()

    def ahead(it, _):
        u, i = it // 2, it % 2
        m = jnp.where(u % 3 == 2, 2, 1 - u % 3)
        h0 = (u // 3) * G + 2 * i
        arrived(_R + 2 * it)
        arrived(_R + 2 * it + 1)
        y = jnp.dot(xtail[...].astype(_F32).reshape(nseg * 8, D), weights(m, [h0, h0 + 1]),
                    preferred_element_type=_F32)
        pre[u, 2 * i] = y[:, 0:128]
        pre[u, 2 * i + 1] = y[:, 128:256]
        relayout(_R + 2 * it, 2)
        return 0
    jax.lax.fori_loop(0, 2 * _NPRE, ahead, 0)

    done, last = _R + 4 * _NPRE, 6 * (ngroup - 1)
    assert 6 * -(-_NPRE // 3) <= _R and done <= last
    for p in range(done, last):
        arrived(p)
    for gi in range(ngroup - 1):
        wo_copy(gi).wait()
    late = None
    for gi in range(ngroup):
        if gi == ngroup - 2:
            for p in range(last, last + 6):
                arrived(p)
            wo_copy(ngroup - 1).wait()
        late = group(None, gi, late)
        for p in range(done, last) if gi == 0 else range(last, last + 6) if gi == ngroup - 2 else ():
            relayout(p, 1)
    out_part(ngroup - 1, 0, D)
    in_copies[5].start()
    for a in range(_R // 2):
        bo_copy(a).start()
    hbuf[M:L, :] = ax[1].astype(_F32)
    hbuf[0:M, :] = acc[0:M, :]

    def step(s, _):
        late = None
        for gi in range(ngroup):
            late = group(s, gi, late)
            if gi == 0:
                emit(s - 1)
        hbuf[M:L, :] = ax[jnp.minimum(s + 1, nseg - 1)].astype(_F32)
        out_part(ngroup - 1, 0, D)
        hbuf[0:M, :] = acc[0:M, :]
        return 0
    def steps(t, _):
        @pl.when(t == 1)
        def _():
            in_copies[5].wait()
        for i in range(3):
            step(1 + 3 * t + i, 0)
        return 0
    assert (nseg - 1) % 3 == 0
    jax.lax.fori_loop(0, (nseg - 1) // 3, steps, 0)
    emit(nseg - 1)

    pltpu.make_async_copy(aout, out_hbm.at[:, :, 0:D], sem_ao).wait()
    for a in range(_R // 2):
        bo_copy(a).wait()


@functools.partial(jax.jit, static_argnames=("A_seg_len",))
def pallas_concat_heads__memory_aug_recurrent_mem_tr__spectral_gfnet__prompt_kernel(
    A_x, A_mem0, A_Wq, A_Wk, A_Wv, A_Wo, A_seg_len, B_x, B_w_r, B_w_i,
):
    _, S, D = A_x.shape
    H, Dh = A_Wq.shape[1], A_Wq.shape[2]
    M = A_mem0.shape[1]
    seg = int(A_seg_len)
    assert (S, D, H, Dh, M, seg) == (2048, 1024, 32, 128, 8, 32) and B_x.shape == (1, S, D)
    L = M + seg
    half = D // 2
    N2 = S // _R
    fo, fe, g = _dft_constants(S, D)
    wr_t, wi_t = B_w_r.T, B_w_i.T

    hbm = pl.BlockSpec(memory_space=pl.ANY)
    vm = pltpu.VMEM
    out = pl.pallas_call(
        functools.partial(_kernel, S=S, D=D, H=H, M=M, seg=seg),
        out_shape=jax.ShapeDtypeStruct((N2, _R, 2 * D), _BF16),
        in_specs=[hbm] * 12,
        out_specs=hbm,
        scratch_shapes=[
            vm((S // seg, seg, D), _BF16),
            vm((S // seg, 8, D), _BF16),
            vm((max(_NPRE, 1), 4, S // seg * 8, Dh), _F32),
            vm((3 * H // 2, D, Dh), _U32),
            vm((3, H, D // 2, Dh), _U32),
            vm((H * Dh // 2, D), _U32),
            vm((L, D), _F32),
            vm((L, H * Dh), _F32),
            vm((L, D), _F32),
            vm((N2, _R, D), _BF16),
            vm((M, D), _BF16),
            vm((1, S), _BF16),
            vm((1, S), _BF16),
            vm((_R // 2, N2, D), _U32),
            vm((_R, half // 2, N2), _U32),
            vm((_R, half // 2, N2), _U32),
            vm((half, half), _BF16),
            vm((half, half // 2), _BF16),
            vm((_R, 2, 2 * N2, N2), _BF16),
            vm((_R, half // 2 + 8, 2 * N2), _F32),
            vm((_R, half // 2, 2 * N2), _F32),
            pltpu.SemaphoreType.DMA((7,)),
            pltpu.SemaphoreType.DMA((_R // 2,)),
            pltpu.SemaphoreType.DMA((_R // 2,)),
            pltpu.SemaphoreType.DMA((3 * H // 2,)),
            pltpu.SemaphoreType.DMA((H // 4,)),
            pltpu.SemaphoreType.DMA,
            pltpu.SemaphoreType.DMA,
        ],
        compiler_params=pltpu.CompilerParams(vmem_limit_bytes=120 * 1024 * 1024),
    )(A_x.reshape(S // seg, seg, D), A_mem0.reshape(M, D), A_Wq, A_Wk, A_Wv, A_Wo.reshape(H * Dh, D),
      B_x.reshape(N2, _R, D), wr_t, wi_t, fo, fe, g)
    return out.reshape(1, S, 2 * D)
```
